```python
import jax
import jax.numpy as jnp

def _softmax(x, axis=-1):
    return jax.nn.softmax(x, axis=axis)
def _gelu(x):
    return jax.nn.gelu(x, approximate=True)
def _silu(x):
    return jax.nn.silu(x)
def _sigmoid(x):
    return jax.nn.sigmoid(x)
def _layernorm(x, axis=-1, eps=1e-5):
    m = jnp.mean(x, axis=axis, keepdims=True)
    v = jnp.var(x, axis=axis, keepdims=True)
    return (x - m) / jnp.sqrt(v + eps)
def _scatter_add(tgt, idx, src, axis=0):
    return tgt.at[idx].add(src)
def _segment_sum(src, seg, n):
    return jax.ops.segment_sum(src, seg, n)
class _Rng:
    def __init__(self, key):
        self._k = key
    def _next(self):
        self._k, sub = jax.random.split(self._k)
        return sub
    def normal(self, shape):
        return jax.random.normal(self._next(), shape, dtype=jnp.bfloat16)
    def randint(self, lo, hi, shape):
        return jax.random.randint(self._next(), shape, lo, hi, dtype=jnp.int32)
    def uniform(self, shape, lo=0.0, hi=1.0):
        return jax.random.uniform(self._next(), shape, jnp.bfloat16, lo, hi)
    def permutation(self, n):
        return jax.random.permutation(self._next(), n)


kernel_name = 'interleave_layers__sliding_local_dilated__glu_gated_glu__prompt'

def setup_inputs():
    _rng = _Rng(jax.random.key(int.from_bytes(__import__("os").urandom(4), "little")))
    _w = (lambda a: (lambda t: t.astype(jnp.bfloat16) if jnp.issubdtype(t.dtype, jnp.floating) else t)(jnp.asarray(a)))
    def _A_setup():
        B, S, D = 1, 2048, 576
        return {
            "x": _w((lambda *s: _rng.normal(s) * 0.05)(B, S, D)),
            "wqkv": _w((lambda *s: _rng.normal(s) * 0.05)(D, 3 * D)),
            "wo": _w((lambda *s: _rng.normal(s) * 0.05)(D, D)),
        }
    _A_in = _A_setup()

    def _B_setup():
        B, S, D, F = 1, 2048, 576, 4608
        return {
            "x": _w((lambda *s: _rng.normal(s) * 0.05)(B, S, D)),
            "w_gate": _w((lambda *s: _rng.normal(s) * 0.05)(D, F)),
            "w_up": _w((lambda *s: _rng.normal(s) * 0.05)(D, F)),
            "w_down": _w((lambda *s: _rng.normal(s) * 0.05)(F, D)),
        }
    _B_in = _B_setup()

    return {
        "A_x": _A_in["x"],
        "A_wqkv": _A_in["wqkv"],
        "A_wo": _A_in["wo"],
        "B_x": _B_in["x"],
        "B_w_gate": _B_in["w_gate"],
        "B_w_up": _B_in["w_up"],
        "B_w_down": _B_in["w_down"],
    }

def reference(A_x, A_wqkv, A_wo, B_x, B_w_gate, B_w_up, B_w_down):
    def _A_ref(x, wqkv, wo):
        B, S, D = x.shape
        H = 32; Dh = D // H
        W, dil = 8, 2
        qkv = (lambda x, *d: x.transpose(*d))((x @ wqkv).reshape(B, S, 3, H, Dh), 2, 0, 3, 1, 4)
        q, k, v = qkv[0], qkv[1], qkv[2]
        scale = Dh ** -0.5
        pos = jnp.arange(S)
        off = jnp.arange(W) * dil
        idx = pos[:, None] - off[None, :]
        mask = idx >= 0
        idx_c = jnp.where(mask, idx, 0).reshape(-1)
        kg = k[:, :, idx_c, :].reshape(B, H, S, W, Dh)
        vg = v[:, :, idx_c, :].reshape(B, H, S, W, Dh)
        logits = jnp.einsum("bhsd,bhswd->bhsw", q, kg) * scale
        logits = jnp.where(mask[None, None, :, :], logits, -1e9)
        attn = _softmax(logits, axis=-1)
        o = jnp.einsum("bhsw,bhswd->bhsd", attn, vg)
        return (lambda x, *d: x.transpose(*d))(o, 0, 2, 1, 3).reshape(B, S, D) @ wo

    def _B_ref(x, w_gate, w_up, w_down):
        g = jnp.einsum("bsd,df->bsf", x, w_gate)
        u = jnp.einsum("bsd,df->bsf", x, w_up)
        h = _sigmoid(g) * u
        return jnp.einsum("bsf,fd->bsd", h, w_down)

    x = A_x
    x = x + _A_ref(_layernorm(x, axis=-1), A_wqkv, A_wo)
    x = x + _B_ref(_layernorm(x, axis=-1), B_w_gate, B_w_up, B_w_down)
    x = x + _A_ref(_layernorm(x, axis=-1), A_wqkv, A_wo)
    x = x + _B_ref(_layernorm(x, axis=-1), B_w_gate, B_w_up, B_w_down)
    return x
```

```python
import jax
import jax.numpy as jnp
import jax.experimental.pallas as pl
import jax.experimental.pallas.tpu as pltpu

S, D, F = 2048, 576, 4608
H, DH, WIN = 32, 18, 8
NT = 16
FC = 512
NCH = F // FC
EPS = 1e-5
f32, bf16, i32 = jnp.float32, jnp.bfloat16, jnp.int32
COLS = [(0, 128), (128, 128), (256, 128), (384, 128), (512, 64)]
ROWS = [(0, 256), (256, 256), (512, 64)]


def _dot(a, b):
    return jnp.dot(a, b, preferred_element_type=f32)


def _cat(xs, axis):
    return xs[0] if len(xs) == 1 else jnp.concatenate(xs, axis=axis)


def _ln(x):
    m = jnp.sum(x, axis=0, keepdims=True) * (1.0 / D)
    xc = x - m
    v = jnp.sum(xc * xc, axis=0, keepdims=True) * (1.0 / D)
    return xc * jax.lax.rsqrt(v + EPS)


def _pair_rows(w):
    return jnp.concatenate([w[0:512], w[64:128], w[512:576], w[0:64], w[512:576]], axis=0)


def _pair_ops(xa, xb):
    b1 = xb[0:64].astype(bf16)
    a9 = xa[512:576].astype(bf16)
    pa = jnp.concatenate([(xa[0:64] - b1.astype(f32)).astype(bf16), xa[64:512].astype(bf16)], axis=0)
    pb = jnp.concatenate([xb[128:512].astype(bf16), xb[64:128].astype(bf16),
                          (xb[512:576] - a9.astype(f32)).astype(bf16)], axis=0)
    pr = jnp.concatenate([b1, a9], axis=0)
    return pa, pb, pr


def _pair_mm(w_ref, pa, pb, pr):
    r = _dot(w_ref[:, 640:768], pr)
    return _dot(w_ref[:, 0:512], pa) + r, _dot(w_ref[:, 128:640], pb) + r


def _kernel(x_hbm, wqkv_hbm, wo_hbm, wg_hbm, wu_hbm, wd_hbm, o_hbm,
            xio, wqkv_raw, wo_raw, wg_raw, wu_raw, wd_raw,
            words, tmp, wqkvT, woT, wguT,
            X, Q, K, V, KS, VS, PA, PB, PR, sems):
    def ffn_copies(c):
        return [
            pltpu.make_async_copy(wg_hbm.at[:, pl.ds(c * FC, FC)], wg_raw.at[c], sems.at[4 + 3 * c]),
            pltpu.make_async_copy(wu_hbm.at[:, pl.ds(c * FC, FC)], wu_raw.at[c], sems.at[5 + 3 * c]),
            pltpu.make_async_copy(wd_hbm.at[:, pl.ds(c * FC, FC)], wd_raw.at[c], sems.at[6 + 3 * c]),
        ]

    cp_wqkv = pltpu.make_async_copy(wqkv_hbm, wqkv_raw, sems.at[0])
    cp_x = pltpu.make_async_copy(x_hbm, xio, sems.at[1])
    cp_wo = pltpu.make_async_copy(wo_hbm, wo_raw, sems.at[2])
    cp_wqkv.start()
    cp_x.start()
    cp_wo.start()

    cp_wqkv.wait()
    wp = _pair_rows(wqkv_raw[...].astype(f32))
    for kt in range(6):
        tmp[kt] = wp[kt * 128:(kt + 1) * 128].T
    for kt in range(6):
        for part in range(3):
            for d in range(DH):
                rows = tmp[kt, pl.ds(part * D + d, H, stride=DH), :]
                wqkvT[pl.ds(part * D + d * H, H), pl.ds(kt * 128, 128)] = rows.astype(bf16)
    cp_x.wait()
    cp_wo.wait()
    for c in range(NCH):
        for cp in ffn_copies(c):
            cp.start()

    for ct, (c0, cw) in enumerate(COLS):
        tmp[ct, pl.ds(0, D), pl.ds(0, cw)] = wo_raw[:, pl.ds(c0, cw)].astype(f32)
    for ct, (c0, cw) in enumerate(COLS):
        rows = jnp.concatenate([tmp[ct, pl.ds(d, H, stride=DH), pl.ds(0, cw)] for d in range(DH)], axis=0)
        woT[pl.ds(c0, cw), :] = _pair_rows(rows).T.astype(bf16)

    for rb, (r0, rn) in enumerate(ROWS):
        words[rb, :, pl.ds(0, rn // 2)] = pltpu.bitcast(xio[pl.ds(r0, rn), :], i32).T
    for t in range(NT):
        p, j = divmod(t, 8)
        for rb, (r0, rn) in enumerate(ROWS):
            wt = words[rb, pl.ds(2 * j + p, 128, stride=16), pl.ds(0, rn // 2)].T
            X[t, pl.ds(r0, rn), :] = pltpu.bitcast(wt, bf16).astype(f32)

    def prep(c, slot):
        wguT[slot, pl.ds(0, FC), :] = _pair_rows(wg_raw[c]).T
        wguT[slot, pl.ds(FC, FC), :] = _pair_rows(wu_raw[c]).T

    lane0 = jax.lax.broadcasted_iota(i32, (H, 128), 1) == 0
    lane0d = jax.lax.broadcasted_iota(i32, (D, 128), 1) == 0

    def qkv(p):
        ops = [_pair_ops(_ln(X[8 * p + i]), _ln(X[8 * p + 4 + i])) for i in range(4)]
        pa, pb, pr = (_cat([o[n] for o in ops], 1) for n in range(3))
        ra, rb = _pair_mm(wqkvT, pa, pb, pr)
        for half, r in enumerate((ra, rb)):
            for i in range(4):
                j = 4 * half + i
                t = 8 * p + j
                cols = slice(i * 128, (i + 1) * 128)
                Q[t] = r[0:D, cols]
                K[t] = r[D:2 * D, cols]
                V[t] = r[2 * D:3 * D, cols]
                if j > 0:
                    KS[t] = pltpu.roll(r[D:2 * D, cols], 1, 1)
                    VS[t] = jnp.where(lane0d, V[0], pltpu.roll(r[2 * D:3 * D, cols], 1, 1))

    def attn(p, j):
        t = 8 * p + j
        q = Q[t]
        logits = []
        for w in range(WIN):
            kt = K[t - w] if j >= w else KS[t - w + 8]
            lg = jnp.sum((q * kt).reshape(DH, H, 128), axis=0) * (DH ** -0.5)
            if j < w:
                lg = jnp.where(lane0, -1e9, lg)
            logits.append(lg)
        m = logits[0]
        for lg in logits[1:]:
            m = jnp.maximum(m, lg)
        es = [jnp.exp(lg - m) for lg in logits]
        den = es[0]
        for e in es[1:]:
            den = den + e
        inv = 1.0 / den
        o = None
        for w in range(WIN):
            vt = V[t - w] if j >= w else VS[t - w + 8]
            term = vt.reshape(DH, H, 128) * (es[w] * inv)[None]
            o = term if o is None else o + term
        return o.reshape(D, 128)

    def out_proj(p):
        ops = [_pair_ops(attn(p, i), attn(p, 4 + i)) for i in range(4)]
        pa, pb, pr = (_cat([o[n] for o in ops], 1) for n in range(3))
        ra, rb = _pair_mm(woT, pa, pb, pr)
        for i in range(4):
            cols = slice(i * 128, (i + 1) * 128)
            xa = X[8 * p + i] + ra[:, cols]
            xb = X[8 * p + 4 + i] + rb[:, cols]
            X[8 * p + i] = xa
            X[8 * p + 4 + i] = xb
            a, b, r = _pair_ops(_ln(xa), _ln(xb))
            PA[p, :, cols] = a
            PB[p, :, cols] = b
            PR[p, :, cols] = r

    def layer(li, carry):
        qkv(0)
        qkv(1)
        out_proj(0)
        out_proj(1)

        @pl.when(li == 0)
        def _():
            for cp in ffn_copies(0):
                cp.wait()
            prep(0, 0)

        def chunk(c, carry2):
            slot = (c + NCH * li) % 2
            nxt = jnp.where(c == NCH - 1, 0, c + 1)

            @pl.when(jnp.logical_and(li == 0, c < NCH - 1))
            def _():
                for cp in ffn_copies(nxt):
                    cp.wait()

            for p in range(2):
                ga, gb = _pair_mm(wguT.at[slot], PA[p], PB[p], PR[p])
                for half, g in enumerate((ga, gb)):
                    h = ((0.5 * jnp.tanh(0.5 * g[0:FC]) + 0.5) * g[FC:2 * FC]).astype(bf16)
                    y = _dot(wd_raw[c], h)
                    for i in range(4):
                        X[8 * p + 4 * half + i] += y[:, i * 128:(i + 1) * 128]
            prep(nxt, 1 - slot)
            return carry2

        jax.lax.fori_loop(0, NCH, chunk, 0)
        return carry

    jax.lax.fori_loop(0, 2, layer, 0)

    for rb, (r0, rn) in enumerate(ROWS):
        for t in range(NT):
            p, j = divmod(t, 8)
            wt = pltpu.bitcast(X[t, pl.ds(r0, rn), :].astype(bf16), i32).T
            words[rb, pl.ds(2 * j + p, 128, stride=16), pl.ds(0, rn // 2)] = wt
        xio[pl.ds(r0, rn), :] = pltpu.bitcast(words[rb, :, pl.ds(0, rn // 2)].T, bf16)
    cp_o = pltpu.make_async_copy(xio, o_hbm, sems.at[3])
    cp_o.start()
    cp_o.wait()


@jax.jit
def pallas_interleave_layers__sliding_local_dilated__glu_gated_glu__prompt_kernel(
    A_x, A_wqkv, A_wo, B_x, B_w_gate, B_w_up, B_w_down,
):
    del B_x
    tile = pltpu.VMEM((NT, D, 128), f32)
    out = pl.pallas_call(
        _kernel,
        out_shape=jax.ShapeDtypeStruct((D, S), bf16),
        in_specs=[pl.BlockSpec(memory_space=pl.ANY)] * 6,
        out_specs=pl.BlockSpec(memory_space=pl.ANY),
        scratch_shapes=[
            pltpu.VMEM((D, S), bf16),
            pltpu.VMEM((D, 3 * D), bf16),
            pltpu.VMEM((D, D), bf16),
            pltpu.VMEM((NCH, D, FC), bf16),
            pltpu.VMEM((NCH, D, FC), bf16),
            pltpu.VMEM((NCH, D, FC), bf16),
            pltpu.VMEM((3, S, 128), i32),
            pltpu.VMEM((6, 3 * D, 128), f32),
            pltpu.VMEM((3 * D, 768), bf16),
            pltpu.VMEM((D, 768), bf16),
            pltpu.VMEM((2, 2 * FC, 768), bf16),
            tile, tile, tile, tile, tile, tile,
            pltpu.VMEM((2, 512, 512), bf16),
            pltpu.VMEM((2, 512, 512), bf16),
            pltpu.VMEM((2, 128, 512), bf16),
            pltpu.SemaphoreType.DMA((4 + 3 * NCH,)),
        ],
        compiler_params=pltpu.CompilerParams(vmem_limit_bytes=120 * 2**20),
        name="interleave",
    )(A_x.reshape(S, D).T, A_wqkv, A_wo, B_w_gate, B_w_up, B_w_down.T)
    return out.T.reshape(1, S, D)
```

```python
import jax
import jax.numpy as jnp
import jax.experimental.pallas as pl
import jax.experimental.pallas.tpu as pltpu

S, D, F = 2048, 576, 4608
H, DH, WIN = 32, 18, 8
NT = 16
FC = 512
NCH = F // FC
HF = FC // 2
HD = D // 2
EPS = 1e-5
f32, bf16, i32 = jnp.float32, jnp.bfloat16, jnp.int32
COLS = [(0, 128), (128, 128), (256, 128), (384, 128), (512, 64)]
ROWS = [(0, 256), (256, 256), (512, 64)]
SC = False
import contextlib
def scope(n):
    return jax.named_scope(n) if SC else contextlib.nullcontext()


def _dot(a, b):
    return jnp.dot(a, b, preferred_element_type=f32)


def _cat(xs, axis):
    return xs[0] if len(xs) == 1 else jnp.concatenate(xs, axis=axis)


def _ln(x):
    m = jnp.sum(x, axis=0, keepdims=True) * (1.0 / D)
    xc = x - m
    v = jnp.sum(xc * xc, axis=0, keepdims=True) * (1.0 / D)
    return xc * jax.lax.rsqrt(v + EPS)


def _pair_rows(w):
    return jnp.concatenate([w[0:512], w[512:576], w[64:128], w[0:64], w[512:576]], axis=0)


def _pair_ops(xa, xb):
    k = xa.shape[0] - 64
    b1 = xb[0:64].astype(bf16)
    a9 = xa[k:].astype(bf16)
    pa = jnp.concatenate([xa[0:64] - b1.astype(f32), xa[64:k]], axis=0).astype(bf16)
    pb = jnp.concatenate([xb[128:k], xb[k:] - a9.astype(f32), xb[64:128]], axis=0).astype(bf16)
    pr = jnp.concatenate([xb[0:64], xa[k:]], axis=0).astype(bf16)
    return pa, pb, pr


def _pair_mm(w, pa, pb, pr):
    k = pa.shape[0]
    r = _dot(w[:, k + 128:k + 256], pr)
    return _dot(w[:, 0:k], pa) + r, _dot(w[:, 128:k + 128], pb) + r


def _glu(c):
    return (0.5 * jnp.tanh(0.5 * c[0:HF]) + 0.5) * c[HF:FC]


def _kernel(x_hbm, wqkv_hbm, wo_hbm, wg_hbm, wu_hbm, wd_hbm, o_hbm,
            xio, wqkv_raw, wo_raw, wg_raw, wu_raw, wd_raw,
            words, tmp, wqkvT, woT, A0,
            X, KE, VE, RS, RA, RB, RR, sems):
    def ffn_copies(c):
        return [
            pltpu.make_async_copy(wg_hbm.at[:, pl.ds(c * FC, FC)], wg_raw.at[c], sems.at[4 + 3 * c]),
            pltpu.make_async_copy(wu_hbm.at[:, pl.ds(c * FC, FC)], wu_raw.at[c], sems.at[5 + 3 * c]),
            pltpu.make_async_copy(wd_hbm.at[:, pl.ds(c * FC, FC)], wd_raw.at[c], sems.at[6 + 3 * c]),
        ]

    cp_wqkv = pltpu.make_async_copy(wqkv_hbm, wqkv_raw, sems.at[0])
    cp_x = pltpu.make_async_copy(x_hbm, xio, sems.at[1])
    cp_wo = pltpu.make_async_copy(wo_hbm, wo_raw, sems.at[2])
    cp_wqkv.start()
    cp_x.start()
    cp_wo.start()

    with scope("w_wqkv"):
        cp_wqkv.wait()
    wp = _pair_rows(wqkv_raw[...].astype(f32))
    for kt in range(6):
        tmp[kt] = wp[kt * 128:(kt + 1) * 128].T
    for kt in range(6):
        for part in range(3):
            for d in range(DH):
                rows = tmp[kt, pl.ds(part * D + d, H, stride=DH), :]
                wqkvT[pl.ds(part * D + d * H, H), pl.ds(kt * 128, 128)] = rows.astype(bf16)
    with scope("w_x"):
        cp_x.wait()
        cp_wo.wait()
    for c in range(NCH):
        for cp in ffn_copies(c):
            cp.start()

    for ct, (c0, cw) in enumerate(COLS):
        tmp[ct, pl.ds(0, D), pl.ds(0, cw)] = wo_raw[:, pl.ds(c0, cw)].astype(f32)
    for ct, (c0, cw) in enumerate(COLS):
        rows = jnp.concatenate([tmp[ct, pl.ds(d, H, stride=DH), pl.ds(0, cw)] for d in range(DH)], axis=0)
        woT[pl.ds(c0, cw), :] = _pair_rows(rows).T.astype(bf16)

    for rb, (r0, rn) in enumerate(ROWS):
        words[rb, :, pl.ds(0, rn // 2)] = pltpu.bitcast(xio[pl.ds(r0, rn), :], i32).T
    for t in range(NT):
        p, j = divmod(t, 8)
        for rb, (r0, rn) in enumerate(ROWS):
            wt = words[rb, pl.ds(2 * j + p, 128, stride=16), pl.ds(0, rn // 2)].T
            X[t, pl.ds(r0, rn), :] = pltpu.bitcast(wt, bf16).astype(f32)

    def tiles_of(res):
        return [r[:, i * 128:(i + 1) * 128] for r in res for i in range(r.shape[1] // 128)]

    def attention(p):
        lane0 = jax.lax.broadcasted_iota(i32, (D, 128), 1) == 0
        ops = [_pair_ops(_ln(X[8 * p + i]), _ln(X[8 * p + 4 + i])) for i in range(4)]
        ops = [_cat([o[n] for o in ops], 1) for n in range(3)]
        for j, k in enumerate(tiles_of(_pair_mm(wqkvT.at[pl.ds(D, D), :], *ops))):
            KE[p, 7 + j] = k
            if j > 0:
                KE[p, j - 1] = pltpu.roll(k, 1, 1)
        ps = []
        for j, q in enumerate(tiles_of(_pair_mm(wqkvT.at[pl.ds(0, D), :], *ops))):
            logits = [None] * WIN
            for d in range(DH):
                for w in range(WIN):
                    t = q[d * H:(d + 1) * H] * KE[p, 7 + j - w, pl.ds(d * H, H), :]
                    logits[w] = t if d == 0 else logits[w] + t
            logits = [lg * (DH ** -0.5) for lg in logits]
            for w in range(j + 1, WIN):
                logits[w] = jnp.where(lane0[0:H], -1e9, logits[w])
            m = logits[0]
            for lg in logits[1:]:
                m = jnp.maximum(m, lg)
            es = [jnp.exp(lg - m) for lg in logits]
            den = es[0]
            for e in es[1:]:
                den = den + e
            inv = 1.0 / den
            ps.append([e * inv for e in es])
        for j, v in enumerate(tiles_of(_pair_mm(wqkvT.at[pl.ds(2 * D, D), :], *ops))):
            VE[p, 7 + j] = v
            if j > 0:
                VE[p, j - 1] = jnp.where(lane0, VE[0, 7], pltpu.roll(v, 1, 1))
        outs = []
        for j in range(8):
            rows = []
            for d in range(DH):
                o = None
                for e in sorted(range(j, j + 8), key=lambda e: (e + 1) % 8):
                    t = ps[j][7 + j - e] * VE[p, e, pl.ds(d * H, H), :]
                    o = t if o is None else o + t
                rows.append(o)
            outs.append(_cat(rows, 0))
        return outs

    def out_proj(p, outs):
        ops = [_pair_ops(outs[i], outs[4 + i]) for i in range(4)]
        ops = [_cat([o[n] for o in ops], 1) for n in range(3)]
        xn = []
        for j, r in enumerate(tiles_of(_pair_mm(woT, *ops))):
            x = X[8 * p + j] + r
            X[8 * p + j] = x
            xn.append(_ln(x))
        short, long_ = [], []
        for i in range(4):
            x1, x2 = xn[2 * i], xn[2 * i + 1]
            b11, b21, t1 = x1[0:256], x1[256:512], x1[512:576]
            b12, b22, t2 = x2[0:256], x2[256:512], x2[512:576]
            t12 = t1 + t2
            short.append([b11 + b22, b12 - b22, b21 - b11])
            long_.append([_cat([b11, t1], 0), _cat([b22, t2], 0),
                          _cat([b11 + b12, t12], 0), _cat([b21 + b22, t12], 0)])
        for n in range(3):
            for i in range(4):
                RS[n, 4 * (i % 2) + 2 * p + i // 2] = short[i][n].astype(bf16)
        for n in range(4):
            for i in range(2):
                g = 2 * p + i
                RA[n, g], RB[n, g], RR[n, g] = _pair_ops(long_[2 * i][n], long_[2 * i + 1][n])

    def blk(c, hrow, hk):
        cols, rows = pl.ds(hrow * HF, HF), pl.ds(hk * 256, 256)
        return _cat([wg_raw[c, rows, cols].T, wu_raw[c, rows, cols].T], 0)

    def ffn_chunk(c, carry):
        low = jax.lax.broadcasted_iota(i32, (FC, 128), 1) < 64

        def tail(hrow):
            cols = pl.ds(hrow * HF, HF)
            tg, tu = wg_raw[c, pl.ds(512, 64), cols], wu_raw[c, pl.ds(512, 64), cols]
            return _cat([_cat([tg, tg], 0).T, _cat([tu, tu], 0).T], 0)

        def short(lhs, n):
            return _dot(lhs, _cat([RS[n, i] for i in range(8)], 1))

        def long_(lhs, t, n):
            lhs = lhs.astype(bf16)
            first = lhs[:, 0:128]
            w = _cat([lhs, jnp.where(low, t, first), jnp.where(low, first, t)], 1)
            ops = [_cat([ref[n, g] for g in range(4)], 1) for ref in (RA, RB, RR)]
            return _cat(list(_pair_mm(w, *ops)), 1)

        a11 = pltpu.bitcast(A0[...], bf16)
        m3 = short(a11, 1)
        a22 = blk(c, 1, 1)
        m4 = short(a22, 2)
        a11, a22 = a11.astype(f32), a22.astype(f32)
        m1 = short((a11 + a22).astype(bf16), 0)
        t1 = tail(0)
        a12 = blk(c, 0, 1).astype(f32)
        m5 = long_(a11 + a12, t1, 1)
        h12 = _glu(m3 + m5)
        m7 = long_(a12 - a22, t1, 3)
        h11 = _glu(m1 + m4 - m5 + m7)
        t2 = tail(1)
        a21 = blk(c, 1, 0).astype(f32)
        m2 = long_(a21 + a22, t2, 0)
        h21 = _glu(m2 + m4)
        m6 = long_(a21 - a11, t2, 2)
        h22 = _glu(m1 - m2 + m3 + m6)
        A0[...] = pltpu.bitcast(blk(jnp.where(c == NCH - 1, 0, c + 1), 0, 0), i32)

        d = {(i, k): wd_raw[c, pl.ds(i * HD, HD), pl.ds(k * HF, HF)] for i in range(2) for k in range(2)}
        d11, d12, d21, d22 = (d[k].astype(f32) for k in ((0, 0), (0, 1), (1, 0), (1, 1)))

        def mm(lhs, rhs):
            return _dot(lhs.astype(bf16), rhs.astype(bf16))

        n2 = mm(d21 + d22, h11)
        n4 = mm(d[1, 1], h21 - h11)
        y21 = n2 + n4
        n6 = mm(d21 - d11, h11 + h12)
        n1 = mm(d11 + d22, h11 + h22)
        n3 = mm(d[0, 0], h12 - h22)
        y22 = n6 - n2 + n1 + n3
        n5 = mm(d11 + d12, h22)
        y12 = n3 + n5
        n7 = mm(d12 - d22, h21 + h22)
        y11 = n1 + n4 - n5 + n7
        for (hr, hc), y in (((1, 0), y21), ((1, 1), y22), ((0, 1), y12), ((0, 0), y11)):
            for i in range(8):
                ab, g = divmod(i, 4)
                X[4 * g + 2 * ab + hc, pl.ds(hr * HD, HD), :] += y[:, i * 128:(i + 1) * 128]
        return carry

    def layer(li, carry):
        with scope("A"):
            o0 = attention(0)
            o1 = attention(1)
            out_proj(0, o0)
            out_proj(1, o1)

        @pl.when(li == 0)
        def _():
            for c in range(NCH):
                for cp in ffn_copies(c):
                    cp.wait()
            A0[...] = pltpu.bitcast(blk(0, 0, 0), i32)

        with scope("ffn"):
            jax.lax.fori_loop(0, NCH, ffn_chunk, 0)
        return carry

    jax.lax.fori_loop(0, 2, layer, 0)

    for rb, (r0, rn) in enumerate(ROWS):
        for t in range(NT):
            p, j = divmod(t, 8)
            wt = pltpu.bitcast(X[t, pl.ds(r0, rn), :].astype(bf16), i32).T
            words[rb, pl.ds(2 * j + p, 128, stride=16), pl.ds(0, rn // 2)] = wt
        xio[pl.ds(r0, rn), :] = pltpu.bitcast(words[rb, :, pl.ds(0, rn // 2)].T, bf16)
    cp_o = pltpu.make_async_copy(xio, o_hbm, sems.at[3])
    with scope("out"):
        cp_o.start()
        cp_o.wait()


@jax.jit
def pallas_interleave_layers__sliding_local_dilated__glu_gated_glu__prompt_kernel(
    A_x, A_wqkv, A_wo, B_x, B_w_gate, B_w_up, B_w_down,
):
    del B_x
    out = pl.pallas_call(
        _kernel,
        out_shape=jax.ShapeDtypeStruct((D, S), bf16),
        in_specs=[pl.BlockSpec(memory_space=pl.ANY)] * 6,
        out_specs=pl.BlockSpec(memory_space=pl.ANY),
        scratch_shapes=[
            pltpu.VMEM((D, S), bf16),
            pltpu.VMEM((D, 3 * D), bf16),
            pltpu.VMEM((D, D), bf16),
            pltpu.VMEM((NCH, D, FC), bf16),
            pltpu.VMEM((NCH, D, FC), bf16),
            pltpu.VMEM((NCH, D, FC), bf16),
            pltpu.VMEM((3, S, 128), i32),
            pltpu.VMEM((6, 3 * D, 128), f32),
            pltpu.VMEM((3 * D, 768), bf16),
            pltpu.VMEM((D, 768), bf16),
            pltpu.VMEM((FC // 2, 256), i32),
            pltpu.VMEM((NT, D, 128), f32),
            pltpu.VMEM((2, 15, D, 128), f32),
            pltpu.VMEM((2, 15, D, 128), f32),
            pltpu.VMEM((3, 8, 256, 128), bf16),
            pltpu.VMEM((4, 4, 256, 128), bf16),
            pltpu.VMEM((4, 4, 256, 128), bf16),
            pltpu.VMEM((4, 4, 128, 128), bf16),
            pltpu.SemaphoreType.DMA((4 + 3 * NCH,)),
        ],
        compiler_params=pltpu.CompilerParams(vmem_limit_bytes=120 * 2**20),
        name="interleave",
    )(A_x.reshape(S, D).T, A_wqkv, A_wo, B_w_gate, B_w_up, B_w_down.T)
    return out.T.reshape(1, S, D)
```

```python
import jax
import jax.numpy as jnp
import jax.experimental.pallas as pl
import jax.experimental.pallas.tpu as pltpu

S, D, F = 2048, 576, 4608
H, DH, WIN = 32, 18, 8
G = 8 * DH
FC = 512
NCH = F // FC
HF = FC // 2
HD = D // 2
XB = 192
NXB = D // XB
WS = 136
EPS = 1e-5
ARR = [1, 2, 3, 4, 5, 6, 7, 0]
RG = 48
f32, bf16, i32 = jnp.float32, jnp.bfloat16, jnp.int32
COLS = [(0, 128), (128, 128), (256, 128), (384, 128), (512, 64)]
LEFT = {1: ((0, 0), 1, (1, 1)), 2: ((1, 0), 1, (1, 1)), 3: ((0, 0),), 4: ((1, 1),),
        5: ((0, 0), 1, (0, 1)), 6: ((1, 0), -1, (0, 0)), 7: ((0, 1), -1, (1, 1))}
RIGHT = {1: ((0, 0), 1, (1, 1)), 2: ((0, 0),), 3: ((0, 1), -1, (1, 1)), 4: ((1, 0), -1, (0, 0)),
         5: ((1, 1),), 6: ((0, 0), 1, (0, 1)), 7: ((1, 0), 1, (1, 1))}
POST = {(0, 0): {1: 1, 4: 1, 5: -1, 7: 1}, (0, 1): {3: 1, 5: 1},
        (1, 0): {2: 1, 4: 1}, (1, 1): {1: 1, 2: -1, 3: 1, 6: 1}}
SC = False
import contextlib
def scope(n):
    return jax.named_scope(n) if SC else contextlib.nullcontext()


def _dot(a, b):
    return jnp.dot(a, b, preferred_element_type=f32)


def _cat(xs, axis):
    return xs[0] if len(xs) == 1 else jnp.concatenate(xs, axis=axis)


def _tree(f, xs):
    while len(xs) > 1:
        xs = [f(xs[i], xs[i + 1]) for i in range(0, len(xs), 2)]
    return xs[0]


def _combine(spec, block):
    if len(spec) == 1:
        return block(*spec[0])
    a, b = block(*spec[0]).astype(f32), block(*spec[2]).astype(f32)
    return a + b if spec[1] > 0 else a - b


def _strassen(order, product):
    acc = {}
    for i in order:
        m = product(i)
        for out, signs in POST.items():
            if i not in signs:
                continue
            if out not in acc:
                acc[out] = (m, signs[i])
            else:
                v, sv = acc[out]
                acc[out] = (v + m, sv) if signs[i] == sv else ((v - m) if sv > 0 else (m - v), 1)
    assert all(sv == 1 for _, sv in acc.values())
    return {out: v for out, (v, _) in acc.items()}


def _moments(x, c):
    xc = x.reshape(x.shape[0] // 16, 16, 128) - c
    return jnp.sum(xc, axis=0), jnp.sum(xc * xc, axis=0)


def _stats(c, s1, s2):
    m = jnp.sum(s1, axis=0, keepdims=True) * (1.0 / D)
    v = jnp.sum(s2, axis=0, keepdims=True) * (1.0 / D) - m * m
    return c + m, jax.lax.rsqrt(jnp.maximum(v, 0.0) + EPS)


def _share_lhs(last, tails, n):
    slot = jax.lax.broadcasted_iota(i32, (last.shape[0] // 2, 128), 1) // (128 // n)
    a, b = pltpu.bitcast(last, i32), pltpu.bitcast(tails, i32)
    return [pltpu.bitcast(jnp.where(slot == k, b, a), bf16) for k in range(n)]


def _share_mm(common, last, variants, rhs, shared):
    r = _dot(variants[0], shared)
    return [_dot(_cat([*common, w], 1), x) + r for w, x in zip([last, *variants[1:]], rhs)]


def _tiles(res):
    return [r[:, i * 128:(i + 1) * 128] for r in res for i in range(r.shape[1] // 128)]


def _kernel(x_hbm, wqkv_hbm, wo_hbm, wg_hbm, wu_hbm, wd_hbm, o_hbm,
            xio, wqkv_raw, wo_raw, wg_raw, wu_raw, wd_raw,
            words, tmp, WT, A0, X0, X1, MOM, ST, K0, K1, KS0, KS1, V0, V1,
            RM, RR, sems, fsems):
    XS, KB, KS, VB = (X0, X1), (K0, K1), (KS0, KS1), (V0, V1)

    def ffn_copies(c):
        return [pltpu.make_async_copy(src.at[:, pl.ds(c * FC, FC)], dst.at[c], fsems.at[3 * c + n])
                for n, (src, dst) in enumerate(((wg_hbm, wg_raw), (wu_hbm, wu_raw), (wd_hbm, wd_raw)))]

    def x_copy(b):
        return pltpu.make_async_copy(x_hbm.at[pl.ds(b * XB, XB), :], xio.at[b], sems.at[b])

    def o_copy(b):
        return pltpu.make_async_copy(xio.at[b], o_hbm.at[pl.ds(b * XB, XB), :], sems.at[b])

    def w_copy(kt):
        rows = pl.ds(*COLS[kt])
        return pltpu.make_async_copy(wqkv_hbm.at[rows, :], wqkv_raw.at[rows, :], sems.at[NXB + kt])

    cp_wo = pltpu.make_async_copy(wo_hbm, wo_raw, sems.at[NXB + 5])
    for b in range(NXB):
        x_copy(b).start()
    cp_wo.start()
    for kt in (4, 3, 0, 1, 2):
        w_copy(kt).start()

    def put_stats(t, st):
        ST[t, 0] = jnp.broadcast_to(st[0], (8, 128))
        ST[t, 1] = jnp.broadcast_to(st[1], (8, 128))

    MOM[...] = jnp.zeros(MOM.shape, f32)

    @pl.loop(0, NXB)
    def _(b):
        with scope("w_x"):
            x_copy(b).wait()
        wt = pltpu.bitcast(xio[b], i32).T
        for s0 in range(0, S, 8):
            l, r0 = divmod(s0, 16)
            words[pl.ds(r0 * WS + l, 8, stride=WS), pl.ds(0, XB // 2)] = wt[s0:s0 + 8]
        for r in range(16):
            x = pltpu.bitcast(words[pl.ds(r * WS, 128), pl.ds(0, XB // 2)].T, bf16).astype(f32)
            XS[r % 2][r // 2, pl.ds(pl.multiple_of(b * XB, XB), XB), :] = x
            c = jnp.where(b == 0, jnp.broadcast_to(x[0:1], (16, 128)), MOM[r, 0])
            s1, s2 = _moments(x, c)
            MOM[r, 0] = c
            MOM[r, 1] += s1
            MOM[r, 2] += s2

    for r in range(16):
        put_stats(8 * (r % 2) + r // 2, _stats(MOM[r, 0, 0:1, :], MOM[r, 1], MOM[r, 2]))

    def permuted(ref, groups, cw=128):
        return _cat([ref[pl.ds(g * G + d, 8, stride=DH), pl.ds(0, cw)] for g in range(groups) for d in range(DH)], 0)

    with scope("w_wo"):
        cp_wo.wait()
    for ct, (c0, cw) in enumerate(COLS):
        tmp[ct, pl.ds(0, D), pl.ds(0, cw)] = wo_raw[:, pl.ds(c0, cw)].astype(f32)
    for ct, (c0, cw) in enumerate(COLS):
        rows = permuted(tmp.at[ct], 4, cw)
        rows = _cat([rows, rows[448:512], rows[384:448], rows[512:576]], 0)
        for kt in range(6):
            WT[kt, pl.ds(3 * D + c0, cw), :] = rows[kt * 128:(kt + 1) * 128].T.astype(bf16)

    for kt in (4, 3, 0, 1, 2):
        with scope("w_wqkv"):
            w_copy(kt).wait()
        w = wqkv_raw[pl.ds(*COLS[kt]), :].astype(f32)
        tmp[kt] = (w if kt < 4 else _cat([w, w], 0)).T
        wt = permuted(tmp.at[kt], 12).astype(bf16)
        WT[kt, pl.ds(0, 3 * D), :] = wt
        if kt == 3:
            WT[4, pl.ds(0, 3 * D), :], WT[5, pl.ds(0, 3 * D), :] = _share_lhs(wt, WT[4, pl.ds(0, 3 * D), :], 2)

    for c in range(NCH):
        for cp in ffn_copies(c):
            cp.start()

    def ln(p, j, rows, z=0):
        x = XS[p][z + j, rows, :]
        return ((x.reshape(-1, 8, 128) - ST[8 * p + j, 0]) * ST[8 * p + j, 1]).reshape(x.shape)

    def project(part, ops):
        w = [WT[kt, pl.ds(part * D, D), :] for kt in range(6)]
        return _tiles(_share_mm(w[0:3], w[3], w[4:6], *ops))

    def pair_tiles(ts):
        xa, xb = _cat(ts[0:4], 1), _cat(ts[4:8], 1)
        ra, rb = xa[512:576].astype(bf16).astype(f32), xb[448:512].astype(bf16).astype(f32)
        pa = _cat([xa[0:448], xa[448:512] - rb], 0).astype(bf16)
        pb = _cat([xb[0:448], xb[512:576] - ra], 0).astype(bf16)
        return [pa, pb], _cat([xa[512:576], xb[448:512]], 0).astype(bf16)

    def attention(p, z, after, first):
        lane0 = jax.lax.broadcasted_iota(i32, (RG, 128), 1) == 0
        if after is not None:
            KB[p][8, 0:8, :] = after
        ops = pair_tiles([ln(p, j, slice(None), z) for j in ARR])
        for j, k in zip(ARR, project(1, ops)):
            for r0 in range(0, D, RG):
                KB[p][j, pl.ds(r0, RG), :] = k[r0:r0 + RG]
                if j > 0:
                    KS[p][j, pl.ds(r0, RG), :] = pltpu.roll(KB[p][z + j, pl.ds(r0, RG), :], 1, 1)
        VB[p][8, 0:8, :] = KS[p][7, D - 8:D, :]
        ps = {}
        for j, q in zip(ARR, project(0, ops)):
            for hg in range(4):
                logits = []
                for w in range(WIN):
                    t = q[hg * G:(hg + 1) * G] * (KB[p] if j >= w else KS[p])[z + (j - w) % 8, pl.ds(hg * G, G), :]
                    lg = jnp.sum(t.reshape(DH, 8, 128), axis=0) * (DH ** -0.5)
                    logits.append(lg if j >= w else jnp.where(lane0[0:8], -1e9, lg))
                m = _tree(jnp.maximum, logits)
                es = [jnp.exp(lg - m) for lg in logits]
                inv = 1.0 / _tree(jnp.add, es)
                ps[j, hg] = [e * inv for e in es]
        vt = dict(zip(ARR, project(2, ops)))
        first = vt[0] if first is None else first
        vs = {}
        for j in ARR[:-1]:
            rows = []
            for r0 in range(0, D, RG):
                VB[p][j, pl.ds(r0, RG), :] = vt[j][r0:r0 + RG]
                sh = pltpu.roll(VB[p][z + j, pl.ds(r0, RG), :], 1, 1)
                if False:
                    sh = jnp.where(lane0, first[r0:r0 + RG], sh)
                rows.append(sh)
            vs[j] = _cat(rows, 0)
        outs = []
        for j in range(8):
            rows = []
            for hg in range(4):
                o = None
                for jj in ARR:
                    v = (vt if jj <= j else vs)[jj][hg * G:(hg + 1) * G]
                    t = v.reshape(DH, 8, 128) * ps[j, hg][(j - jj) % 8]
                    o = t if o is None else o + t
                rows.append(o.reshape(G, 128))
            outs.append(_cat(rows, 0))
        return outs, vs[7][D - 8:D], first

    def out_proj(p, outs):
        for j, r in enumerate(project(3, pair_tiles(outs))):
            x = XS[p][j] + r
            XS[p][j] = x
            put_stats(8 * p + j, _stats(x[0:1], *_moments(x, x[0:1])))

    def right_operands(p, g, r0):
        blocks = {(hk, hc): ln(p, 2 * g + hc, pl.ds(hk * HD + r0, 32)) for hk in range(2) for hc in range(2)}
        return {i: _combine(spec, lambda *k: blocks[k]) for i, spec in RIGHT.items()}

    def gate_up_left(c, i):
        out = []
        for ref in (wg_raw, wu_raw):
            w = _combine(LEFT[i], lambda hr, hk: ref[c, pl.ds(hk * HD, HD), pl.ds(hr * HF, HF)]).astype(bf16)
            out.append(_cat([w[0:256]] + [w[256:HD]] * 4, 0).T)
        return _cat([w[r:r + 16] for r in range(0, HF, 16) for w in out], 0)

    def ffn_chunk(c, carry):
        def gate_up(i):
            w = pltpu.bitcast(A0[...], bf16) if i == 3 else gate_up_left(c + (c >> (4 + i)), i)
            rhs = [_cat([RM[i - 1, 2 * g], RM[i - 1, 2 * g + 1]], 1) for g in range(4)]
            last = w[:, 128:256]
            return _cat(_share_mm([w[:, 0:128]], last, _share_lhs(last, w[:, 256:384], 4),
                                  rhs, _cat([RR[i - 1, 0], RR[i - 1, 1]], 1)), 1)

        def glu(gu):
            gu = gu.reshape(HF // 16, 2, 16, S // 2)
            return ((0.5 * jnp.tanh(0.5 * gu[:, 0]) + 0.5) * gu[:, 1]).reshape(HF, S // 2)

        h = {k: glu(v) for k, v in _strassen((3, 4, 1, 5, 7, 2, 6), gate_up).items()}
        A0[...] = pltpu.bitcast(gate_up_left(jnp.where(c == NCH - 1, 0, c + 1), 3), i32)

        def down(i):
            cc = c + (c >> (4 + i))
            w = _combine(LEFT[i], lambda hr, hk: wd_raw[cc, pl.ds(hr * HD, HD), pl.ds(hk * HF, HF)])
            return _dot(w.astype(bf16), _combine(RIGHT[i], lambda *k: h[k]).astype(bf16))

        for (hr, hc), y in _strassen((2, 4, 6, 1, 3, 5, 7), down).items():
            for i in range(8):
                g, p = divmod(i, 2)
                XS[p][2 * g + hc, pl.ds(hr * HD, HD), :] += y[:, i * 128:(i + 1) * 128]
        return carry

    def fake(c, carry):
        X0[c, 0:256] += RM[c, c].astype(f32)
        X0[c, 0:128] += RR[c, c].astype(f32)
        X0[c, 0:256] += A0[:, 0:128].astype(f32) + A0[:, 128:256].astype(f32) + A0[:, 256:384].astype(f32)
        return carry

    @pl.loop(0, 2)
    def _(li):
        with scope("A"):
            z = li >> 4
            o0, last, first = attention(0, z, None, None)
            o1, _, _ = attention(1, z, last, first)
            out_proj(0, o0)
            out_proj(1, o1)

        with scope("operands"):
            @pl.loop(0, 5)
            def _(s):
                r0 = pl.multiple_of(s * 32, 32)
                for p in range(2):
                    for g in range(4):
                        for i, v in right_operands(p, g, r0).items():
                            RM[i - 1, 2 * g + p, pl.ds(r0, 32), :] = v.astype(bf16)

            for k in range(4):
                for p in range(2):
                    src = 256 if k == 0 else 128 + 32 * k
                    own = {i: v.astype(bf16) for i, v in right_operands(p, k, src).items()}
                    for i, v in own.items():
                        RR[i - 1, p, pl.ds(32 * k, 32), :] = v
                    for g in range(4):
                        if g != k:
                            for i, v in right_operands(p, g, src).items():
                                RM[i - 1, 2 * g + p, pl.ds(128 + 32 * (k or g), 32), :] = (
                                    v - own[i].astype(f32)).astype(bf16)

        @pl.when(li == 0)
        def _():
            for c in range(NCH):
                for cp in ffn_copies(c):
                    cp.wait()
            A0[...] = pltpu.bitcast(gate_up_left(0, 3), i32)

        with scope("ffn"):
            jax.lax.fori_loop(0, NCH, ffn_chunk, 0)

        @pl.when(li == 0)
        def _():
            with scope("stats"):
                for p in range(2):
                    for j in range(8):
                        x = XS[p][j]
                        put_stats(8 * p + j, _stats(x[0:1], *_moments(x, x[0:1])))

        @pl.when(li == 1)
        def _():
            with scope("out"):
                @pl.loop(0, NXB)
                def _(b):
                    for r in range(16):
                        x = XS[r % 2][r // 2, pl.ds(pl.multiple_of(b * XB, XB), XB), :]
                        words[pl.ds(r * WS, 128), pl.ds(0, XB // 2)] = pltpu.bitcast(x.astype(bf16), i32).T
                    wt = _cat([words[pl.ds((s0 % 16) * WS + s0 // 16, 8, stride=WS), pl.ds(0, XB // 2)]
                               for s0 in range(0, S, 8)], 0)
                    xio[b] = pltpu.bitcast(wt.T, bf16)
                    o_copy(b).start()

                for b in range(NXB):
                    o_copy(b).wait()


@jax.jit
def pallas_interleave_layers__sliding_local_dilated__glu_gated_glu__prompt_kernel(
    A_x, A_wqkv, A_wo, B_x, B_w_gate, B_w_up, B_w_down,
):
    del B_x
    out = pl.pallas_call(
        _kernel,
        out_shape=jax.ShapeDtypeStruct((D, S), bf16),
        in_specs=[pl.BlockSpec(memory_space=pl.ANY)] * 6,
        out_specs=pl.BlockSpec(memory_space=pl.ANY),
        scratch_shapes=[
            pltpu.VMEM((NXB, XB, S), bf16),
            pltpu.VMEM((D, 3 * D), bf16),
            pltpu.VMEM((D, D), bf16),
            pltpu.VMEM((NCH, D, FC), bf16),
            pltpu.VMEM((NCH, D, FC), bf16),
            pltpu.VMEM((NCH, D, FC), bf16),
            pltpu.VMEM((16 * WS, 128), i32),
            pltpu.VMEM((5, 3 * D, 128), f32),
            pltpu.VMEM((6, 4 * D, 128), bf16),
            pltpu.VMEM((FC // 2, 384), i32),
            pltpu.VMEM((8, D, 128), f32),
            pltpu.VMEM((8, D, 128), f32),
            pltpu.VMEM((16, 3, 16, 128), f32),
            pltpu.VMEM((16, 2, 8, 128), f32),
            *[pltpu.VMEM((9, D, 128), f32)] * 6,
            pltpu.VMEM((7, 8, 256, 128), bf16),
            pltpu.VMEM((7, 2, 128, 128), bf16),
            pltpu.SemaphoreType.DMA((NXB + 6,)),
            pltpu.SemaphoreType.DMA((3 * NCH,)),
        ],
        compiler_params=pltpu.CompilerParams(vmem_limit_bytes=120 * 2**20),
        name="interleave",
    )(A_x.reshape(S, D).T, A_wqkv, A_wo, B_w_gate, B_w_up, B_w_down.T)
    return out.T.reshape(1, S, D)
```

```python
import jax
import jax.numpy as jnp
import jax.experimental.pallas as pl
import jax.experimental.pallas.tpu as pltpu

S, D, F = 2048, 576, 4608
DH, WIN = 18, 8
G = 8 * DH
HD = D // 2
FC = 512
HF = FC // 2
NCH = F // FC
XB = 192
NXB = D // XB
EPS = 1e-5
QKV_TILES = (1, 2, 3, 4, 5, 6, 7, 0)
OUT_TILES = (0, 7, 6, 1, 5, 2, 4, 3)
f32, bf16, i32 = jnp.float32, jnp.bfloat16, jnp.int32

LEFT = {1: ((0, 0), 1, (1, 1)), 2: ((1, 0), 1, (1, 1)), 3: ((0, 0),), 4: ((1, 1),),
        5: ((0, 0), 1, (0, 1)), 6: ((1, 0), -1, (0, 0)), 7: ((0, 1), -1, (1, 1))}
RIGHT = {1: ((0, 0), 1, (1, 1)), 2: ((0, 0),), 3: ((0, 1), -1, (1, 1)), 4: ((1, 0), -1, (0, 0)),
         5: ((1, 1),), 6: ((0, 0), 1, (0, 1)), 7: ((1, 0), 1, (1, 1))}
POST = {(0, 0): {1: 1, 4: 1, 5: -1, 7: 1}, (0, 1): {3: 1, 5: 1},
        (1, 0): {2: 1, 4: 1}, (1, 1): {1: 1, 2: -1, 3: 1, 6: 1}}
ORDER = (3, 5, 2, 4, 1, 7, 6)


def _dot(a, b):
    return jnp.dot(a, b, preferred_element_type=f32)


def _cat(xs, axis):
    return jnp.concatenate(xs, axis=axis)


def _tree(f, xs):
    while len(xs) > 1:
        xs = [f(xs[i], xs[i + 1]) for i in range(0, len(xs), 2)]
    return xs[0]


def _tiles(xs):
    return [x[:, i * 128:(i + 1) * 128] for x in xs for i in range(x.shape[1] // 128)]


def _combine(spec, block):
    if len(spec) == 1:
        return block(*spec[0])
    a, b = block(*spec[0]).astype(f32), block(*spec[2]).astype(f32)
    return a + b if spec[1] > 0 else a - b


def _strassen(product):
    acc = {}
    for i in ORDER:
        m = product(i)
        for out, signs in POST.items():
            if i not in signs:
                continue
            if out not in acc:
                acc[out] = (m, signs[i])
            else:
                v, sv = acc[out]
                acc[out] = (v + m, sv) if signs[i] == sv else ((v - m) if sv > 0 else (m - v), 1)
    assert all(sv == 1 for _, sv in acc.values())
    return {out: v for out, (v, _) in acc.items()}


def _share_lhs(last, tails, n):
    slot = jax.lax.broadcasted_iota(i32, (last.shape[0] // 2, 128), 1) // (128 // n)
    a, b = pltpu.bitcast(last, i32), pltpu.bitcast(tails, i32)
    return [pltpu.bitcast(jnp.where(slot == k, b, a), bf16) for k in range(n)]


def _share_mm(common, last, variants, rhs, shared):
    r = _dot(variants[0], shared)
    return [_dot(_cat([*common, w], 1), x) + r for w, x in zip([last, *variants[1:]], rhs)]


def _moments(x, c):
    xc = x.reshape(x.shape[0] // 16, 16, 128) - c
    return jnp.sum(xc, axis=0), jnp.sum(xc * xc, axis=0)


def _kernel(x_hbm, wqkv_hbm, wo_hbm, wg_hbm, wu_hbm, wd_hbm, o_hbm,
            xio, wqkv_raw, wo_raw, wg_raw, wu_raw, wd_raw, words, tmp,
            WT, A0, XP, FILL, MOM, ST, RM, RR, HS, sems):
    def xrows(r0, n):
        return pl.ds(XB + r0, n)

    def ffn_copies():
        return [pltpu.make_async_copy(src.at[:, pl.ds(c * FC, FC)], dst.at[c], sems.at[11])
                for c in range(NCH)
                for src, dst in ((wg_hbm, wg_raw), (wu_hbm, wu_raw), (wd_hbm, wd_raw))]

    def x_copy(b, n):
        return pltpu.make_async_copy(x_hbm.at[pl.ds(b * 128, n), :], xio.at[b, pl.ds(0, n), :], sems.at[b])

    def w_copy(kt, n):
        rows = pl.ds(pl.multiple_of(kt * 128, 128), n)
        return pltpu.make_async_copy(wqkv_hbm.at[rows, :], wqkv_raw.at[rows, :], sems.at[5 + kt])

    def o_copy(b, part):
        n = 64 if part else 128
        return pltpu.make_async_copy(xio.at[2 * b + part, pl.ds(0, n), :],
                                     o_hbm.at[pl.ds(b * XB + part * 128, n), :], sems.at[2 * b + part])

    wo_copy = pltpu.make_async_copy(wo_hbm, wo_raw, sems.at[10])
    x_copy(4, 64).start()
    for b in range(4):
        x_copy(b, 128).start()
    w_copy(4, 64).start()
    wo_copy.start()
    for kt in (3, 0, 1, 2):
        w_copy(kt, 128).start()

    FILL[...] = jnp.zeros(FILL.shape, f32)

    @pl.loop(0, 8)
    def _(j):
        XP[:, j, 0:XB, :] = jnp.zeros((2, XB, 128), f32)

    def load_rows(b, n, first):
        x_copy(b, n).wait()
        words[0, 0:S // 2, 0:n] = pltpu.bitcast(xio[b, pl.ds(0, n), :].T, i32)
        for j in range(8):
            pair = words[0, pl.ds(j, 128, stride=8), pl.ds(0, n)].T
            for p, bits in enumerate((pair << 16, pair & -65536)):
                x = pltpu.bitcast(bits, f32)
                XP[p, j, xrows(pl.multiple_of(b * 128, 128), n), :] = x
                t = 8 * p + j
                if first:
                    MOM[t, 0] = c = jnp.broadcast_to(x[0:1], (16, 128))
                    MOM[t, 1], MOM[t, 2] = _moments(x, c)
                else:
                    s1, s2 = _moments(x, MOM[t, 0])
                    MOM[t, 1] += s1
                    MOM[t, 2] += s2

    def store_rows(b, part, xs):
        n = 64 if part else 128
        for j in range(8):
            lo, hi = (pltpu.bitcast(xs[8 * p + j][part * 128:part * 128 + n].astype(bf16).astype(f32), i32)
                      for p in range(2))
            words[part, pl.ds(j, 128, stride=8), pl.ds(0, n)] = (jax.lax.shift_right_logical(lo, 16) | hi).T
        xio[2 * b + part, pl.ds(0, n), :] = pltpu.bitcast(words[part, 0:S // 2, 0:n], bf16).T

    def regroup(t, groups, n):
        return _cat([tmp[t, pl.ds(g * G + d, 8, stride=DH), pl.ds(0, n)]
                     for g in range(groups) for d in range(DH)], 0)

    def prepare_wqkv(kt, n=128, last=False):
        w_copy(kt, n).wait()
        w = wqkv_raw[pl.ds(pl.multiple_of(kt * 128, 128), n), :]
        tmp[0, 0:3 * D, :] = _cat([w] * (128 // n), 0).astype(f32).T
        wt = regroup(0, 12, 128).astype(bf16)
        WT[kt, pl.ds(0, 3 * HD), :] = pltpu.bitcast(wt, i32)
        if last:
            for k, v in enumerate(_share_lhs(wt, pltpu.bitcast(WT[4, pl.ds(0, 3 * HD), :], bf16), 2)):
                WT[4 + k, pl.ds(0, 3 * HD), :] = pltpu.bitcast(v, i32)

    def prepare_wo():
        wo_copy.wait()
        cols = [(ct, min(128, D - ct * 128)) for ct in range(5)]
        for ct, n in cols:
            tmp[ct, 0:D, 0:n] = wo_raw[:, pl.ds(ct * 128, n)].astype(f32)
        for ct, n in cols:
            rows = regroup(ct, 4, n)
            rows = _cat([rows, rows[448:512], rows[384:448], rows[512:576]], 0)
            for kt in range(6):
                WT[kt, pl.ds(3 * HD + ct * 64, n // 2), :] = pltpu.bitcast(
                    rows[kt * 128:(kt + 1) * 128].T.astype(bf16), i32)

    load_rows(4, 64, True)
    pl.loop(0, 4)(lambda b: load_rows(b, 128, False))
    prepare_wqkv(4, 64)
    prepare_wo()
    prepare_wqkv(3, last=True)
    pl.loop(0, 3)(prepare_wqkv)
    for cp in ffn_copies():
        cp.start()

    def put_stats(t, c, s1, s2):
        m = jnp.sum(s1, axis=0, keepdims=True) * (1.0 / D)
        v = jnp.sum(s2, axis=0, keepdims=True) * (1.0 / D) - m * m
        ST[t, 0] = jnp.broadcast_to(c + m, (8, 128))
        ST[t, 1] = jnp.broadcast_to(jax.lax.rsqrt(jnp.maximum(v, 0.0) + EPS), (8, 128))

    def normed(p, j, r0, n):
        x = XP[p, j, xrows(r0, n), :].reshape(n // 8, 8, 128)
        return ((x - ST[8 * p + j, 0]) * ST[8 * p + j, 1]).reshape(n, 128)

    def pair_tiles(ts):
        xa, xb = _cat(ts[0:4], 1), _cat(ts[4:8], 1)
        ra, rb = xa[512:576].astype(bf16).astype(f32), xb[448:512].astype(bf16).astype(f32)
        pa = _cat([xa[0:448], xa[448:512] - rb], 0).astype(bf16)
        pb = _cat([xb[0:448], xb[512:576] - ra], 0).astype(bf16)
        return [pa, pb], _cat([xa[512:576], xb[448:512]], 0).astype(bf16)

    def project(r0, n, ops):
        w = [pltpu.bitcast(WT[kt, pl.ds(r0 // 2, n // 2), :], bf16) for kt in range(6)]
        return _tiles(_share_mm(w[0:3], w[3], w[4:6], *ops))

    def attention(p):
        lane = jax.lax.broadcasted_iota(i32, (8, 128), 1)

        def lane_is(at, after):
            return lane + (pltpu.bitcast(after[D - 8:D], i32) & (p >> 4)) == at

        ops = pair_tiles([normed(p, j, 0, D) for j in QKV_TILES])
        kt = dict(zip(QKV_TILES, project(D, D, ops)))
        ks = {j: pltpu.roll(kt[j], 1, 1) for j in range(1, 8)}
        v_hi = project(2 * D + HD, HD, ops)
        probs = {}
        for j, q in zip(QKV_TILES, project(0, D, ops)):
            for hg in range(4):
                logits = []
                for w in range(WIN):
                    t = q[hg * G:(hg + 1) * G] * (kt if j >= w else ks)[(j - w) % 8][hg * G:(hg + 1) * G]
                    lg = jnp.sum(t.reshape(DH, 8, 128), axis=0) * (DH ** -0.5)
                    logits.append(lg if j >= w else jnp.where(lane == 0, -1e9, lg))
                m = _tree(jnp.maximum, logits)
                es = [jnp.exp(lg - m) for lg in logits]
                inv = 1.0 / _tree(jnp.add, es)
                if j < 7:
                    es[j] = es[j] + jnp.where(lane + p == 0, (7 - j) * es[7], 0.0)
                probs[j, hg] = [e * inv for e in es]
        vt = {j: _cat([lo, hi], 0) for j, lo, hi in zip(QKV_TILES, project(2 * D, HD, ops), v_hi)}
        vs, after = {}, ks[7]
        for j in range(1, 8):
            t = jnp.where(lane_is(127, after), FILL[...].reshape(D // 8, 8, 128), vt[j].reshape(D // 8, 8, 128))
            vs[j] = after = pltpu.roll(t.reshape(D, 128), 1, 1)
        t = jnp.where(lane_is(-p, after), vt[0].reshape(D // 8, 8, 128), 0.0)
        FILL[...] = pltpu.roll(t.reshape(D, 128), 127, 1)
        outs = []
        for j in range(8):
            rows = []
            for hg in range(4):
                o = None
                for jj in QKV_TILES:
                    v = (vt if jj <= j else vs)[jj][hg * G:(hg + 1) * G]
                    t = v.reshape(DH, 8, 128) * probs[j, hg][(j - jj) % 8]
                    o = t if o is None else o + t
                rows.append(o.reshape(G, 128))
            outs.append(_cat(rows, 0))
        for j, r in zip(OUT_TILES, project(3 * D, D, pair_tiles([outs[j] for j in OUT_TILES]))):
            XP[p, j, xrows(0, D), :] = x = XP[p, j, xrows(0, D), :] + r
            put_stats(8 * p + j, x[0:1], *_moments(x, x[0:1]))

    def right_operands(p, g, r0):
        blocks = {(hk, hc): normed(p, 2 * g + hc, hk * HD + r0, 32) for hk in range(2) for hc in range(2)}
        return {i: _combine(spec, lambda *k: blocks[k]) for i, spec in RIGHT.items()}

    def prepare_ffn_input():
        @pl.loop(0, 5)
        def _(s):
            r0 = pl.multiple_of(s * 32, 32)
            for p in range(2):
                for g in range(4):
                    for i, v in right_operands(p, g, r0).items():
                        RM[i - 1, 2 * g + p, pl.ds(r0, 32), :] = v.astype(bf16)

        for k in range(4):
            for p in range(2):
                src = 256 if k == 0 else 128 + 32 * k
                own = {i: v.astype(bf16) for i, v in right_operands(p, k, src).items()}
                for i, v in own.items():
                    RR[i - 1, p, pl.ds(32 * k, 32), :] = v
                for g in range(4):
                    if g != k:
                        for i, v in right_operands(p, g, src).items():
                            RM[i - 1, 2 * g + p, pl.ds(128 + 32 * (k or g), 32), :] = (
                                v - own[i].astype(f32)).astype(bf16)

    def gate_up_left(c, i):
        out = []
        for ref in (wg_raw, wu_raw):
            w = _combine(LEFT[i], lambda hr, hk: ref[c, pl.ds(hk * HD, HD), pl.ds(hr * HF, HF)]).astype(bf16)
            out.append(_cat([w[0:256]] + [w[256:HD]] * 4, 0).T)
        return _cat([w[r:r + 16] for r in range(0, HF, 16) for w in out], 0)

    def gate_up(c):
        def product(i):
            w = pltpu.bitcast(A0[...], bf16) if i == ORDER[0] else gate_up_left(c + (c >> (4 + i)), i)
            rhs = [_cat([RM[i - 1, 2 * g], RM[i - 1, 2 * g + 1]], 1) for g in range(4)]
            last = w[:, 128:256]
            return _cat(_share_mm([w[:, 0:128]], last, _share_lhs(last, w[:, 256:384], 4),
                                  rhs, _cat([RR[i - 1, 0], RR[i - 1, 1]], 1)), 1)

        def glu(gu):
            gu = gu.reshape(HF // 16, 2, 16, S // 2)
            return ((0.5 * jnp.tanh(0.5 * gu[:, 0]) + 0.5) * gu[:, 1]).reshape(HF, S // 2)

        h = {k: glu(v) for k, v in _strassen(product).items()}
        for i, spec in RIGHT.items():
            for t, v in enumerate(_tiles([_combine(spec, lambda *k: h[k])])):
                HS[i - 1, t, pl.ds(pl.multiple_of(c * HF, HF), HF), :] = v.astype(bf16)
        A0[...] = pltpu.bitcast(gate_up_left(jnp.where(c == NCH - 1, 0, c + 1), ORDER[0]), i32)

    def down(b):
        n = XB // 2
        r0 = pl.multiple_of(b * XB, XB)

        def product(i):
            z = b >> (4 + i)
            w = _combine(LEFT[i], lambda hr, hk: _cat(
                [wd_raw[c + z, pl.ds(r0 + hr * n, n), pl.ds(hk * HF, HF)] for c in range(NCH)], 1))
            return _dot(w.astype(bf16), _cat([HS[i - 1, t] for t in range(8)], 1))

        win = XP.at[:, :, pl.ds(r0, 2 * XB), :]
        finished = [win[t // 8, t % 8, 0:XB, :] for t in range(16)]
        seen = []
        for (hr, hc), y in _strassen(product).items():
            for i in range(8):
                g, p = divmod(i, 2)
                j, rows = 2 * g + hc, pl.ds(XB + hr * n, n)
                win[p, j, rows, :] = x = win[p, j, rows, :] + y[:, i * 128:(i + 1) * 128]
                t = 8 * p + j
                c, s1, s2 = MOM[t, 0], MOM[t, 1], MOM[t, 2]
                if t not in seen:
                    seen.append(t)
                    MOM[t, 0] = c = jnp.where(b == 0, jnp.broadcast_to(x[0:1], (16, 128)), c)
                    s1, s2 = jnp.where(b == 0, 0.0, s1), jnp.where(b == 0, 0.0, s2)
                u1, u2 = _moments(x, c)
                MOM[t, 1], MOM[t, 2] = s1 + u1, s2 + u2
        return finished

    @pl.loop(0, 2)
    def _(layer):
        for t in range(16):
            put_stats(t, MOM[t, 0, 0:1, :], MOM[t, 1], MOM[t, 2])
        pl.loop(0, 2)(attention)

        @pl.when(layer == 0)
        def _():
            for cp in ffn_copies():
                cp.wait()
            A0[...] = pltpu.bitcast(gate_up_left(0, ORDER[0]), i32)

        prepare_ffn_input()
        pl.loop(0, NCH)(gate_up)

        @pl.loop(0, NXB)
        def _(b):
            prev = jnp.maximum(b - 1, 0)
            finished = down(b)
            for part in range(2):
                store_rows(prev, part, finished)

            @pl.when(jnp.logical_and(layer == 1, b > 0))
            def _():
                for part in range(2):
                    o_copy(prev, part).start()

    for part in range(2):
        store_rows(NXB - 1, part, [XP[t // 8, t % 8, xrows(D - XB, XB), :] for t in range(16)])
        o_copy(NXB - 1, part).start()
    for b in range(NXB):
        for part in range(2):
            o_copy(b, part).wait()


@jax.jit
def pallas_interleave_layers__sliding_local_dilated__glu_gated_glu__prompt_kernel(
    A_x: jax.Array,
    A_wqkv: jax.Array,
    A_wo: jax.Array,
    B_x: jax.Array,
    B_w_gate: jax.Array,
    B_w_up: jax.Array,
    B_w_down: jax.Array,
):
    del B_x
    out = pl.pallas_call(
        _kernel,
        out_shape=jax.ShapeDtypeStruct((D, S), bf16),
        in_specs=[pl.BlockSpec(memory_space=pl.ANY)] * 6,
        out_specs=pl.BlockSpec(memory_space=pl.ANY),
        scratch_shapes=[
            pltpu.VMEM((6, 128, S), bf16),
            pltpu.VMEM((D, 3 * D), bf16),
            pltpu.VMEM((D, D), bf16),
            pltpu.VMEM((NCH, D, FC), bf16),
            pltpu.VMEM((NCH, D, FC), bf16),
            pltpu.VMEM((NCH, D, FC), bf16),
            pltpu.VMEM((2, S // 2 + 32, 128), i32),
            pltpu.VMEM((5, 3 * D + 32, 128), f32),
            pltpu.VMEM((6, 4 * HD, 128), i32),
            pltpu.VMEM((FC // 2, 384), i32),
            pltpu.VMEM((2, 8, XB + D, 128), f32),
            pltpu.VMEM((D, 128), f32),
            pltpu.VMEM((16, 3, 16, 128), f32),
            pltpu.VMEM((16, 2, 8, 128), f32),
            pltpu.VMEM((7, 8, 256, 128), bf16),
            pltpu.VMEM((7, 2, 128, 128), bf16),
            pltpu.VMEM((7, 8, F // 2, 128), bf16),
            pltpu.SemaphoreType.DMA((12,)),
        ],
        compiler_params=pltpu.CompilerParams(vmem_limit_bytes=110 * 2**20),
        name="interleave",
    )(A_x.reshape(S, D).T, A_wqkv, A_wo, B_w_gate, B_w_up, B_w_down.T)
    return out.T.reshape(1, S, D)
```

```python
import jax
import jax.numpy as jnp
import jax.experimental.pallas as pl
import jax.experimental.pallas.tpu as pltpu

S, D, F = 2048, 576, 4608
DH, WIN = 18, 8
G = 8 * DH
HD = D // 2
KB = D // 3
FT = 128
FC = 3 * FT
NCH = F // FC
XB = 192
NXB = D // XB
EPS = 1e-5
QKV_TILES = (1, 2, 3, 4, 5, 6, 7, 0)
OUT_TILES = (0, 7, 6, 1, 5, 2, 4, 3)
f32, bf16, i32 = jnp.float32, jnp.bfloat16, jnp.int32

RHO = 3 ** 0.5


def _scheme():
    out = {}
    for i in range(3):
        j, k = (i + 1) % 3, (i + 2) % 3
        for name, left, right, res in (
                ("a", [(1, i, j)], [(1, j, j), (-1, j, i)], [(1, i, i), (1, j, i)]),
                ("b", [(1, j, i)], [(1, i, i), (-1, i, j)], [(-1, j, j), (-1, i, j)]),
                ("c", [(1, i, j), (1, j, i)], [(1, i, j), (1, j, i)], [(-1, i, j), (1, j, i)]),
                ("d", [(1, i, i), (1, i, j), (-1, k, i)], [(1, j, i)], [(-1, i, k)]),
                ("e", [(1, i, i), (-1, j, i), (1, i, k)], [(1, k, i)], [(1, i, j)])):
            right = sorted(((-s if f == 2 else s, f, n) for s, f, n in right), key=lambda t: -t[0])
            if right[0][0] < 0:
                right, res = ([(-s, u, v) for s, u, v in ts] for ts in (right, res))
            out[name + str(i)] = (left, right, res)
    return out


SCHEME = _scheme()
STAGES = (("a0", "b0", "d0", "c0", "a2", "b2", "c2", "e0"), ("d1", "a1", "b1", "c1", "e1"), ("d2", "e2"))
PRODUCTS = [n for st in STAGES for n in st]
STAGED = 2


def _passes():
    order = []

    def run(t, g, stage):
        for n in STAGES[stage]:
            if (t, 2, n) not in order:
                order.append((t, 2, n))
            order.append((t, g, n))

    def shared(t, count):
        todo = [(t, 2, n) for n in PRODUCTS if t < 4 and (t, 2, n) not in order]
        order.extend(todo[:count])

    for t in range(4):
        run(t, 0, 0), run(t, 0, 1), shared(t + 1, 2), run(t, 0, 2)
        run(t, 1, 0), shared(t + 1, 1), run(t, 1, 1), shared(t + 1, 4), run(t, 1, 2)
    return order


def _dot(a, b):
    return jnp.dot(a, b, preferred_element_type=f32)


def _cat(xs, axis):
    return jnp.concatenate(xs, axis=axis)


def _tree(f, xs):
    while len(xs) > 1:
        xs = [f(xs[i], xs[i + 1]) for i in range(0, len(xs), 2)]
    return xs[0]


def _tiles(xs):
    return [x[:, i * 128:(i + 1) * 128] for x in xs for i in range(x.shape[1] // 128)]


def _combine(terms, block):
    v = block(*terms[0][1:])
    for s, *at in terms[1:]:
        v, w = v.astype(f32), block(*at).astype(f32)
        v = v + w if s > 0 else v - w
    return v


def _forms(x, y):
    return [x + y, x - y, x + x]


def _signed_sum(terms):
    s, v = terms[-1]
    for t, m in terms[-2::-1]:
        s, v = (s, v + m) if t == s else (1, v - m if s > 0 else m - v)
    return s, v


def _results(products):
    acc = {}
    for n, m in products:
        for s, i, d in SCHEME[n][2]:
            acc.setdefault((i, d), []).append((s, m))
    out = []
    for i in range(3):
        a = [_signed_sum(acc[i, d]) for d in range(3)]
        neg = [(-s, v) for s, v in a]
        x = _signed_sum([a[0], neg[1]])
        y = _signed_sum([_signed_sum([a[2], neg[1]]), _signed_sum([neg[0], a[2]])])
        assert x[0] == 1 and y[0] == 1
        out.append((x[1], y[1]))
    return out


def _share_lhs(last, tails, n):
    slot = jax.lax.broadcasted_iota(i32, (last.shape[0] // 2, 128), 1) // (128 // n)
    a, b = pltpu.bitcast(last, i32), pltpu.bitcast(tails, i32)
    return [pltpu.bitcast(jnp.where(slot == k, b, a), bf16) for k in range(n)]


def _share_mm(common, last, variants, rhs, shared):
    r = _dot(variants[0], shared)
    return [_dot(_cat([*common, w], 1), x) + r for w, x in zip([last, *variants[1:]], rhs)]


def _moments(x, c):
    xc = x.reshape(x.shape[0] // 16, 16, 128) - c
    return jnp.sum(xc, axis=0), jnp.sum(xc * xc, axis=0)


def _kernel(x_hbm, wqkv_hbm, wo_hbm, wg_hbm, wu_hbm, wd_hbm, o_hbm,
            xio, wqkv_raw, wo_raw, wg_raw, wu_raw, wd_raw, words, tmp,
            WT, A0, XP, FILL, MOM, ST, RM, HS, sems):
    def xrows(r0, n):
        return pl.ds(XB + r0, n)

    def ffn_copies():
        return [pltpu.make_async_copy(src.at[:, pl.ds(c * FC, FC)], dst.at[c], sems.at[11])
                for c in range(NCH)
                for src, dst in ((wg_hbm, wg_raw), (wu_hbm, wu_raw), (wd_hbm, wd_raw))]

    def x_copy(b, n):
        return pltpu.make_async_copy(x_hbm.at[pl.ds(b * 128, n), :], xio.at[b, pl.ds(0, n), :], sems.at[b])

    def w_copy(kt, n):
        rows = pl.ds(pl.multiple_of(kt * 128, 128), n)
        return pltpu.make_async_copy(wqkv_hbm.at[rows, :], wqkv_raw.at[rows, :], sems.at[5 + kt])

    def o_copy(b, part):
        k, n = 2 * b + part, XB // 2
        return pltpu.make_async_copy(xio.at[k, pl.ds(0, n), :], o_hbm.at[pl.ds(k * n, n), :], sems.at[k])

    wo_copy = pltpu.make_async_copy(wo_hbm, wo_raw, sems.at[10])
    x_copy(4, 64).start()
    for b in range(4):
        x_copy(b, 128).start()
    w_copy(4, 64).start()
    wo_copy.start()
    for kt in (3, 0, 1, 2):
        w_copy(kt, 128).start()

    FILL[...] = jnp.zeros(FILL.shape, f32)

    @pl.loop(0, 8)
    def _(j):
        XP[:, j, 0:XB, :] = jnp.zeros((2, XB, 128), f32)

    def load_rows(b, n, first):
        x_copy(b, n).wait()
        words[0, 0:S // 2, 0:n] = pltpu.bitcast(xio[b, pl.ds(0, n), :].T, i32)
        for j in range(8):
            pair = words[0, pl.ds(j, 128, stride=8), pl.ds(0, n)].T
            for p, bits in enumerate((pair << 16, pair & -65536)):
                x = pltpu.bitcast(bits, f32)
                XP[p, j, xrows(pl.multiple_of(b * 128, 128), n), :] = x
                t = 8 * p + j
                if first:
                    MOM[t, 0] = c = jnp.broadcast_to(x[0:1], (16, 128))
                    MOM[t, 1], MOM[t, 2] = _moments(x, c)
                else:
                    s1, s2 = _moments(x, MOM[t, 0])
                    MOM[t, 1] += s1
                    MOM[t, 2] += s2

    def store_rows(b, part, xs):
        n = XB // 2
        for j in range(8):
            lo, hi = (pltpu.bitcast(xs[8 * p + j].astype(bf16).astype(f32), i32) for p in range(2))
            words[part, pl.ds(j, 128, stride=8), pl.ds(0, n)] = (jax.lax.shift_right_logical(lo, 16) | hi).T
        xio[2 * b + part, pl.ds(0, n), :] = pltpu.bitcast(words[part, 0:S // 2, 0:n], bf16).T

    def regroup(t, groups, n):
        return _cat([tmp[t, pl.ds(g * G + d, 8, stride=DH), pl.ds(0, n)]
                     for g in range(groups) for d in range(DH)], 0)

    def prepare_wqkv(kt, n=128, last=False):
        w_copy(kt, n).wait()
        w = wqkv_raw[pl.ds(pl.multiple_of(kt * 128, 128), n), :]
        tmp[0, 0:3 * D, :] = _cat([w] * (128 // n), 0).astype(f32).T
        wt = regroup(0, 12, 128).astype(bf16)
        WT[kt, pl.ds(0, 3 * HD), :] = pltpu.bitcast(wt, i32)
        if last:
            for k, v in enumerate(_share_lhs(wt, pltpu.bitcast(WT[4, pl.ds(0, 3 * HD), :], bf16), 2)):
                WT[4 + k, pl.ds(0, 3 * HD), :] = pltpu.bitcast(v, i32)

    def prepare_wo():
        wo_copy.wait()
        cols = [(ct, min(128, D - ct * 128)) for ct in range(5)]
        for ct, n in cols:
            tmp[ct, 0:D, 0:n] = wo_raw[:, pl.ds(ct * 128, n)].astype(f32)
        for ct, n in cols:
            rows = regroup(ct, 4, n)
            rows = _cat([rows, rows[448:512], rows[384:448], rows[512:576]], 0)
            for kt in range(6):
                WT[kt, pl.ds(3 * HD + ct * 64, n // 2), :] = pltpu.bitcast(
                    rows[kt * 128:(kt + 1) * 128].T.astype(bf16), i32)

    load_rows(4, 64, True)
    pl.loop(0, 4)(lambda b: load_rows(b, 128, False))
    prepare_wqkv(4, 64)
    prepare_wo()
    prepare_wqkv(3, last=True)
    pl.loop(0, 3)(prepare_wqkv)
    for cp in ffn_copies():
        cp.start()

    def put_stats(t, c, s1, s2, scale=1.0):
        m = jnp.sum(s1, axis=0, keepdims=True) * (1.0 / D)
        v = jnp.sum(s2, axis=0, keepdims=True) * (1.0 / D) - m * m
        ST[t, 0] = jnp.broadcast_to(c + m, (8, 128))
        ST[t, 1] = jnp.broadcast_to(jax.lax.rsqrt(jnp.maximum(v, 0.0) + EPS) * scale, (8, 128))

    def normed(p, j, r0, n):
        x = XP[p, j, xrows(r0, n), :].reshape(n // 8, 8, 128)
        return ((x - ST[8 * p + j, 0]) * ST[8 * p + j, 1]).reshape(n, 128)

    def pair_tiles(ts):
        xa, xb = _cat(ts[0:4], 1), _cat(ts[4:8], 1)
        ra, rb = xa[512:576].astype(bf16).astype(f32), xb[448:512].astype(bf16).astype(f32)
        pa = _cat([xa[0:448], xa[448:512] - rb], 0).astype(bf16)
        pb = _cat([xb[0:448], xb[512:576] - ra], 0).astype(bf16)
        return [pa, pb], _cat([xa[512:576], xb[448:512]], 0).astype(bf16)

    def project(r0, n, ops):
        w = [pltpu.bitcast(WT[kt, pl.ds(r0 // 2, n // 2), :], bf16) for kt in range(6)]
        return _tiles(_share_mm(w[0:3], w[3], w[4:6], *ops))

    def attention(p):
        lane = jax.lax.broadcasted_iota(i32, (8, 128), 1)

        def lane_is(at, after):
            return lane + (pltpu.bitcast(after[D - 8:D], i32) & (p >> 4)) == at

        ops = pair_tiles([normed(p, j, 0, D) for j in QKV_TILES])
        kt = dict(zip(QKV_TILES, project(D, D, ops)))
        ks = {j: pltpu.roll(kt[j], 1, 1) for j in range(1, 8)}
        v_hi = project(2 * D + HD, HD, ops)
        probs = {}
        for j, q in zip(QKV_TILES, project(0, D, ops)):
            for hg in range(4):
                logits = []
                for w in range(WIN):
                    t = q[hg * G:(hg + 1) * G] * (kt if j >= w else ks)[(j - w) % 8][hg * G:(hg + 1) * G]
                    lg = jnp.sum(t.reshape(DH, 8, 128), axis=0) * (DH ** -0.5)
                    logits.append(lg if j >= w else jnp.where(lane == 0, -1e9, lg))
                m = _tree(jnp.maximum, logits)
                es = [jnp.exp(lg - m) for lg in logits]
                inv = 1.0 / _tree(jnp.add, es)
                if j < 7:
                    es[j] = es[j] + jnp.where(lane + p == 0, (7 - j) * es[7], 0.0)
                probs[j, hg] = [e * inv for e in es]
        vt = {j: _cat([lo, hi], 0) for j, lo, hi in zip(QKV_TILES, project(2 * D, HD, ops), v_hi)}
        vs, after = {}, ks[7]
        for j in range(1, 8):
            t = jnp.where(lane_is(127, after), FILL[...].reshape(D // 8, 8, 128), vt[j].reshape(D // 8, 8, 128))
            vs[j] = after = pltpu.roll(t.reshape(D, 128), 1, 1)
        t = jnp.where(lane_is(-p, after), vt[0].reshape(D // 8, 8, 128), 0.0)
        FILL[...] = pltpu.roll(t.reshape(D, 128), 127, 1)
        outs = []
        for j in range(8):
            rows = []
            for hg in range(4):
                o = None
                for jj in QKV_TILES:
                    v = (vt if jj <= j else vs)[jj][hg * G:(hg + 1) * G]
                    t = v.reshape(DH, 8, 128) * probs[j, hg][(j - jj) % 8]
                    o = t if o is None else o + t
                rows.append(o.reshape(G, 128))
            outs.append(_cat(rows, 0))
        for j, r in zip(OUT_TILES, project(3 * D, D, pair_tiles([outs[j] for j in OUT_TILES]))):
            XP[p, j, xrows(0, D), :] = x = XP[p, j, xrows(0, D), :] + r
            put_stats(8 * p + j, x[0:1], *_moments(x, x[0:1]), scale=0.5 * RHO if j % 2 else 0.5)

    def right_operands(p, t, r0):
        fs = [_forms(*(normed(p, 2 * t + hc, k * KB + r0, 16) for hc in range(2))) for k in range(3)]
        return [_combine(SCHEME[n][1], lambda f, k: fs[k][f]) for n in PRODUCTS]

    def prepare_ffn_input(i):
        r = pl.multiple_of(i * 16, 16)
        for t in range(4):
            for p in range(2):
                for q, v in enumerate(right_operands(p, t, r)):
                    RM[q, p, t, pl.ds(r, 16), :] = v.astype(bf16)
                src = r + 64 * (2 - p)
                for q, (own, v) in enumerate(zip(right_operands(p, t, src), right_operands(1 - p, t, src))):
                    RM[q, 2, t, pl.ds(r + 64 * p, 16), :] = own.astype(bf16)
                    RM[q, 1 - p, t, pl.ds(r + 64, 16), :] = (
                        v - RM[q, 2, t, pl.ds(r + 64 * p, 16), :].astype(f32)).astype(bf16)

    def gate_up_left(c, n):
        out = []
        for ref in (wg_raw, wu_raw):
            w = _combine(SCHEME[n][0], lambda i, k: ref[c, pl.ds(k * KB, KB), pl.ds(i * FT, FT)]).astype(bf16)
            out.append(_cat([w, w[128:KB]], 0).T)
        return _cat([w[r:r + 16] for r in range(0, FT, 16) for w in out], 0)

    def stage_left(c):
        for q in range(STAGED):
            A0[q] = pltpu.bitcast(gate_up_left(c, PRODUCTS[q]), i32)

    def gate_up(c):
        def glu(gu, scale):
            gu = gu.reshape(FT // 16, 2, 16, 128)
            return ((0.25 * jnp.tanh(scale * gu[:, 0]) + 0.25) * gu[:, 1]).reshape(FT, 128)

        left = {}
        for q, n in enumerate(PRODUCTS):
            w = pltpu.bitcast(A0[q], bf16) if q < STAGED else gate_up_left(c + (c >> (5 + q)), n)
            both, second = _share_lhs(w[:, 0:128], w[:, 128:256], 2)
            left[n] = (w[:, 0:128], second, both)
        shared, products = {}, {}
        for t, g, n in _passes():
            m = _dot(left[n][g], RM[PRODUCTS.index(n), g, t])
            if g == 2:
                shared[t, n] = m
            else:
                products.setdefault((t, g), []).append((n, m + shared[t, n]))
        for (t, g), ms in products.items():
            fs = [_forms(glu(x, 0.5), glu(y, 0.5 / RHO)) for x, y in _results(ms)]
            for q, n in enumerate(PRODUCTS):
                HS[q, 4 * g + t, pl.ds(pl.multiple_of(c * FT, FT), FT), :] = _combine(
                    SCHEME[n][1], lambda f, k: fs[k][f]).astype(bf16)
        stage_left(jnp.where(c == NCH - 1, 0, c + 1))

    def down(b):
        n = XB // 3
        r0 = pl.multiple_of(b * XB, XB)
        left = []
        for q, name in enumerate(PRODUCTS):
            z = b >> (5 + q)
            left.append(_combine(SCHEME[name][0], lambda i, k: _cat(
                [wd_raw[c + z, pl.ds(r0 + i * n, n), pl.ds(k * FT, FT)] for c in range(NCH)], 1)).astype(bf16))
        win = XP.at[:, :, pl.ds(r0, 2 * XB), :]
        finished = [win[t // 8, t % 8, 0:XB, :] for t in range(16)]
        cuts = (0, 4, 5, 6, 7, 8)
        for u0, u1 in zip(cuts[:-1], cuts[1:]):
            res = _results([(name, _dot(left[q], _cat([HS[q, u] for u in range(u0, u1)], 1)))
                            for q, name in enumerate(PRODUCTS)])
            for hc in range(2):
                y = _cat([ys[hc] for ys in res], 0)
                for u, dx in zip(range(u0, u1), _tiles([y * (1 / RHO) if hc else y])):
                    p, j = u // 4, 2 * (u % 4) + hc
                    win[p, j, XB:2 * XB, :] = x = win[p, j, XB:2 * XB, :] + dx
                    t = 8 * p + j
                    MOM[t, 0] = c = jnp.where(b == 0, jnp.broadcast_to(x[0:1], (16, 128)), MOM[t, 0])
                    for k, part in enumerate(_moments(x, c)):
                        MOM[t, 1 + k] = jnp.where(b == 0, 0.0, MOM[t, 1 + k]) + part
        return finished

    @pl.loop(0, 2)
    def _(layer):
        for t in range(16):
            put_stats(t, MOM[t, 0, 0:1, :], MOM[t, 1], MOM[t, 2])
        pl.loop(0, 2)(attention)

        @pl.when(layer == 0)
        def _():
            for cp in ffn_copies():
                cp.wait()
            stage_left(0)

        pl.loop(0, 4)(prepare_ffn_input)
        pl.loop(0, NCH)(gate_up)

        @pl.loop(0, NXB)
        def _(b):
            prev = jnp.maximum(b - 1, 0)
            finished = down(b)
            for part in range(2):
                store_rows(prev, part, [x[part * XB // 2:(part + 1) * XB // 2] for x in finished])

            @pl.when(jnp.logical_and(layer == 1, b > 0))
            def _():
                for part in range(2):
                    o_copy(prev, part).start()

    @pl.loop(0, 2)
    def _(part):
        rows = xrows(pl.multiple_of(D - XB + part * (XB // 2), XB // 2), XB // 2)
        store_rows(NXB - 1, part, [XP[t // 8, t % 8, rows, :] for t in range(16)])
        o_copy(NXB - 1, part).start()

    for b in range(NXB):
        for part in range(2):
            o_copy(b, part).wait()


@jax.jit
def pallas_interleave_layers__sliding_local_dilated__glu_gated_glu__prompt_kernel(
    A_x: jax.Array,
    A_wqkv: jax.Array,
    A_wo: jax.Array,
    B_x: jax.Array,
    B_w_gate: jax.Array,
    B_w_up: jax.Array,
    B_w_down: jax.Array,
):
    del B_x
    out = pl.pallas_call(
        _kernel,
        out_shape=jax.ShapeDtypeStruct((D, S), bf16),
        in_specs=[pl.BlockSpec(memory_space=pl.ANY)] * 6,
        out_specs=pl.BlockSpec(memory_space=pl.ANY),
        scratch_shapes=[
            pltpu.VMEM((6, 128, S), bf16),
            pltpu.VMEM((D, 3 * D), bf16),
            pltpu.VMEM((D, D), bf16),
            pltpu.VMEM((NCH, D, FC), bf16),
            pltpu.VMEM((NCH, D, FC), bf16),
            pltpu.VMEM((NCH, D, FC), bf16),
            pltpu.VMEM((2, S // 2 + 32, 128), i32),
            pltpu.VMEM((5, 3 * D + 32, 128), f32),
            pltpu.VMEM((6, 4 * HD, 128), i32),
            pltpu.VMEM((STAGED, FT, 256), i32),
            pltpu.VMEM((2, 8, XB + D, 128), f32),
            pltpu.VMEM((D, 128), f32),
            pltpu.VMEM((16, 3, 16, 128), f32),
            pltpu.VMEM((16, 2, 8, 128), f32),
            pltpu.VMEM((15, 3, 4, 128, 128), bf16),
            pltpu.VMEM((15, 8, F // 3, 128), bf16),
            pltpu.SemaphoreType.DMA((12,)),
        ],
        compiler_params=pltpu.CompilerParams(vmem_limit_bytes=120 * 2**20),
        name="interleave",
    )(A_x.reshape(S, D).T, A_wqkv, A_wo, B_w_gate, B_w_up, B_w_down.T)
    return out.T.reshape(1, S, D)
```

```python
import jax
import jax.numpy as jnp
import jax.experimental.pallas as pl
import jax.experimental.pallas.tpu as pltpu

S, D, F = 2048, 576, 4608
DH, WIN = 18, 8
G = 8 * DH
HD = D // 2
KB = D // 3
FT = 128
FC = 3 * FT
NCH = F // FC
XB = 192
NXB = D // XB
EPS = 1e-5
TINY = 1e-30
QKV_TILES = (1, 2, 3, 4, 5, 6, 7, 0)
OUT_TILES = (0, 7, 6, 1, 5, 2, 4, 3)
f32, bf16, i32 = jnp.float32, jnp.bfloat16, jnp.int32

RHO = 3 ** 0.5


def _scheme():
    out = {}
    for i in range(3):
        j, k = (i + 1) % 3, (i + 2) % 3
        for name, left, right, res in (
                ("a", [(1, i, j)], [(1, j, j), (-1, j, i)], [(1, i, i), (1, j, i)]),
                ("b", [(1, j, i)], [(1, i, i), (-1, i, j)], [(-1, j, j), (-1, i, j)]),
                ("c", [(1, i, j), (1, j, i)], [(1, i, j), (1, j, i)], [(-1, i, j), (1, j, i)]),
                ("d", [(1, i, i), (1, i, j), (-1, k, i)], [(1, j, i)], [(-1, i, k)]),
                ("e", [(1, i, i), (-1, j, i), (1, i, k)], [(1, k, i)], [(1, i, j)])):
            right = sorted(((-s if f == 2 else s, f, n) for s, f, n in right), key=lambda t: -t[0])
            if right[0][0] < 0:
                right, res = ([(-s, u, v) for s, u, v in ts] for ts in (right, res))
            out[name + str(i)] = (left, right, res)
    return out


SCHEME = _scheme()
STAGES = (("a0", "b0", "d0", "c0", "a2", "b2", "c2", "e0"), ("d1", "a1", "b1", "c1", "e1"), ("d2", "e2"))
PRODUCTS = [n for st in STAGES for n in st]
STAGED = 2


def _passes():
    order = []

    def run(t, g, stage):
        for n in STAGES[stage]:
            if (t, 2, n) not in order:
                order.append((t, 2, n))
            order.append((t, g, n))

    def shared(t, count):
        todo = [(t, 2, n) for n in PRODUCTS if t < 4 and (t, 2, n) not in order]
        order.extend(todo[:count])

    for t in range(4):
        run(t, 0, 0), run(t, 0, 1), shared(t + 1, 2), run(t, 0, 2)
        run(t, 1, 0), shared(t + 1, 1), run(t, 1, 1), shared(t + 1, 4), run(t, 1, 2)
    return order


def _dot(a, b):
    return jnp.dot(a, b, preferred_element_type=f32)


def _cat(xs, axis):
    return jnp.concatenate(xs, axis=axis)


def _tree(f, xs):
    while len(xs) > 1:
        xs = [f(xs[i], xs[i + 1]) for i in range(0, len(xs), 2)]
    return xs[0]


def _tiles(xs):
    return [x[:, i * 128:(i + 1) * 128] for x in xs for i in range(x.shape[1] // 128)]


def _combine(terms, block):
    v = block(*terms[0][1:])
    for s, *at in terms[1:]:
        v, w = v.astype(f32), block(*at).astype(f32)
        v = v + w if s > 0 else v - w
    return v


def _forms(x, y):
    return [x + y, x - y, x + x]


def _signed_sum(terms):
    s, v = terms[-1]
    for t, m in terms[-2::-1]:
        s, v = (s, v + m) if t == s else (1, v - m if s > 0 else m - v)
    return s, v


def _results(products):
    acc = {}
    for n, m in products:
        for s, i, d in SCHEME[n][2]:
            acc.setdefault((i, d), []).append((s, m))
    out = []
    for i in range(3):
        a = [_signed_sum(acc[i, d]) for d in range(3)]
        neg = [(-s, v) for s, v in a]
        x = _signed_sum([a[0], neg[1]])
        y = _signed_sum([_signed_sum([a[2], neg[1]]), _signed_sum([neg[0], a[2]])])
        assert x[0] == 1 and y[0] == 1
        out.append((x[1], y[1]))
    return out


def _share_lhs(last, tails, n):
    slot = jax.lax.broadcasted_iota(i32, (last.shape[0] // 2, 128), 1) // (128 // n)
    a, b = pltpu.bitcast(last, i32), pltpu.bitcast(tails, i32)
    return [pltpu.bitcast(jnp.where(slot == k, b, a), bf16) for k in range(n)]


def _share_mm(common, last, variants, rhs, shared):
    r = _dot(variants[0], shared)
    return [_dot(_cat([*common, w], 1), x) + r for w, x in zip([last, *variants[1:]], rhs)]


def _moments(x, c):
    xc = x.reshape(x.shape[0] // 16, 16, 128) - c
    return jnp.sum(xc, axis=0), jnp.sum(xc * xc, axis=0)


def _kernel(x_hbm, wqkv_hbm, wo_hbm, wg_hbm, wu_hbm, wd_hbm, o_hbm,
            xio, wqkv_raw, wo_raw, wg_raw, wu_raw, wd_raw, words, tmp,
            WT, A0, XP, FILL, MOM, ST, RM, HS, sems):
    def xrows(r0, n):
        return pl.ds(XB + r0, n)

    def ffn_copies():
        return [pltpu.make_async_copy(src.at[:, pl.ds(c * FC, FC)], dst.at[c], sems.at[11])
                for c in range(NCH)
                for src, dst in ((wg_hbm, wg_raw), (wu_hbm, wu_raw), (wd_hbm, wd_raw))]

    def x_copy(b, n):
        return pltpu.make_async_copy(x_hbm.at[pl.ds(b * 128, n), :], xio.at[b, pl.ds(0, n), :], sems.at[b])

    def w_copy(kt, n):
        rows = pl.ds(pl.multiple_of(kt * 128, 128), n)
        return pltpu.make_async_copy(wqkv_hbm.at[rows, :], wqkv_raw.at[rows, :], sems.at[5 + kt])

    def o_copy(b, part):
        k, n = 2 * b + part, XB // 2
        return pltpu.make_async_copy(xio.at[k, pl.ds(0, n), :], o_hbm.at[pl.ds(k * n, n), :], sems.at[k])

    wo_copy = pltpu.make_async_copy(wo_hbm, wo_raw, sems.at[10])
    x_copy(4, 64).start()
    for b in range(4):
        x_copy(b, 128).start()
    w_copy(4, 64).start()
    wo_copy.start()
    for kt in (3, 0, 1, 2):
        w_copy(kt, 128).start()

    FILL[...] = jnp.zeros(FILL.shape, f32)

    @pl.loop(0, 8)
    def _(j):
        XP[:, j, 0:XB, :] = jnp.zeros((2, XB, 128), f32)

    def load_rows(b, n, first):
        x_copy(b, n).wait()
        words[0, 0:S // 2, 0:n] = pltpu.bitcast(xio[b, pl.ds(0, n), :].T, i32)
        for j in range(8):
            pair = words[0, pl.ds(j, 128, stride=8), pl.ds(0, n)].T
            for p, bits in enumerate((pair << 16, pair & -65536)):
                x = pltpu.bitcast(bits, f32)
                XP[p, j, xrows(pl.multiple_of(b * 128, 128), n), :] = x
                t = 8 * p + j
                if first:
                    MOM[t, 0] = c = jnp.broadcast_to(x[0:1], (16, 128))
                    MOM[t, 1], MOM[t, 2] = _moments(x, c)
                else:
                    s1, s2 = _moments(x, MOM[t, 0])
                    MOM[t, 1] += s1
                    MOM[t, 2] += s2

    def store_rows(b, part, xs):
        n = XB // 2
        for j in range(8):
            lo, hi = (pltpu.bitcast(xs[8 * p + j].astype(bf16).astype(f32), i32) for p in range(2))
            words[part, pl.ds(j, 128, stride=8), pl.ds(0, n)] = (jax.lax.shift_right_logical(lo, 16) | hi).T
        xio[2 * b + part, pl.ds(0, n), :] = pltpu.bitcast(words[part, 0:S // 2, 0:n], bf16).T

    def regroup(t, groups, n):
        return _cat([tmp[t, pl.ds(g * G + d, 8, stride=DH), pl.ds(0, n)]
                     for g in range(groups) for d in range(DH)], 0)

    def prepare_wqkv(kt, n=128, last=False):
        w_copy(kt, n).wait()
        w = wqkv_raw[pl.ds(pl.multiple_of(kt * 128, 128), n), :]
        tmp[0, 0:3 * D, :] = _cat([w] * (128 // n), 0).astype(f32).T
        wt = regroup(0, 12, 128).astype(bf16)
        WT[kt, pl.ds(0, 3 * HD), :] = pltpu.bitcast(wt, i32)
        if last:
            for k, v in enumerate(_share_lhs(wt, pltpu.bitcast(WT[4, pl.ds(0, 3 * HD), :], bf16), 2)):
                WT[4 + k, pl.ds(0, 3 * HD), :] = pltpu.bitcast(v, i32)

    def prepare_wo():
        wo_copy.wait()
        cols = [(ct, min(128, D - ct * 128)) for ct in range(5)]
        for ct, n in cols:
            tmp[ct, 0:D, 0:n] = wo_raw[:, pl.ds(ct * 128, n)].astype(f32)
        for ct, n in cols:
            rows = regroup(ct, 4, n)
            rows = _cat([rows, rows[448:512], rows[384:448], rows[512:576]], 0)
            for kt in range(6):
                WT[kt, pl.ds(3 * HD + ct * 64, n // 2), :] = pltpu.bitcast(
                    rows[kt * 128:(kt + 1) * 128].T.astype(bf16), i32)

    load_rows(4, 64, True)
    pl.loop(0, 4)(lambda b: load_rows(b, 128, False))
    prepare_wqkv(4, 64)
    prepare_wo()
    prepare_wqkv(3, last=True)
    pl.loop(0, 3)(prepare_wqkv)
    for cp in ffn_copies():
        cp.start()

    def put_stats(t, slot, scale, c, s1, s2):
        m = jnp.sum(s1, axis=0, keepdims=True) * (1.0 / D)
        v = jnp.maximum(jnp.sum(s2, axis=0, keepdims=True) * (1.0 / D) - m * m, 0.0)
        unit = jax.lax.rsqrt(v + TINY)
        ST[t, 0] = jnp.broadcast_to(c + m, (8, 128))
        ST[t, 1] = jnp.broadcast_to(unit * scale, (8, 128))
        ST[t, slot] = jnp.broadcast_to((v + TINY) * unit * jax.lax.rsqrt(v + EPS), (8, 128))

    def normed(p, j, r0, n):
        x = XP[p, j, xrows(r0, n), :].reshape(n // 8, 8, 128)
        return ((x - ST[8 * p + j, 0]) * ST[8 * p + j, 1]).reshape(n, 128)

    def pair_tiles(ts):
        xa, xb = _cat(ts[0:4], 1), _cat(ts[4:8], 1)
        ra, rb = xa[512:576].astype(bf16).astype(f32), xb[448:512].astype(bf16).astype(f32)
        pa = _cat([xa[0:448], xa[448:512] - rb], 0).astype(bf16)
        pb = _cat([xb[0:448], xb[512:576] - ra], 0).astype(bf16)
        return [pa, pb], _cat([xa[512:576], xb[448:512]], 0).astype(bf16)

    def project(r0, n, ops):
        w = [pltpu.bitcast(WT[kt, pl.ds(r0 // 2, n // 2), :], bf16) for kt in range(6)]
        return _tiles(_share_mm(w[0:3], w[3], w[4:6], *ops))

    def attention(p):
        lane = jax.lax.broadcasted_iota(i32, (8, 128), 1)

        def lane_is(at, after):
            return lane + (pltpu.bitcast(after[D - 8:D], i32) & (p >> 4)) == at

        ops = pair_tiles([normed(p, j, 0, D) for j in QKV_TILES])
        kt = dict(zip(QKV_TILES, project(D, D, ops)))
        ks = {j: pltpu.roll(kt[j], 1, 1) for j in range(1, 8)}
        v_hi = project(2 * D + HD, HD, ops)
        gt = [ST[8 * p + j, 2] for j in range(8)]
        gz = {j: jnp.where(lane == 0, 0.0, pltpu.roll(gt[j], 1, 1)) for j in range(1, 8)}
        gs = {j: jnp.where(lane == 0, ST[0, 2], g) for j, g in gz.items()}
        probs, peak = {}, {}
        for j, q in zip(QKV_TILES, project(0, D, ops)):
            gains = [(gt if j >= w else gs)[(j - w) % 8] for w in range(WIN)]
            scales = [g * (gt[j] * DH ** -0.5) for g in gains]
            peak[j] = _tree(jnp.maximum, [(gt if j >= w else gz)[(j - w) % 8] for w in range(WIN)])
            gains = [g * (1.0 / peak[j]) for g in gains]
            for hg in range(4):
                logits = []
                for w in range(WIN):
                    t = q[hg * G:(hg + 1) * G] * (kt if j >= w else ks)[(j - w) % 8][hg * G:(hg + 1) * G]
                    lg = jnp.sum(t.reshape(DH, 8, 128), axis=0) * scales[w]
                    logits.append(lg if j >= w else jnp.where(lane == 0, -1e9, lg))
                m = _tree(jnp.maximum, logits)
                es = [jnp.exp(lg - m) for lg in logits]
                inv = 1.0 / _tree(jnp.add, es)
                if j < 7:
                    es[j] = es[j] + jnp.where(lane + p == 0, (7 - j) * es[7], 0.0)
                probs[j, hg] = [e * inv * g for e, g in zip(es, gains)]
        vt = {j: _cat([lo, hi], 0) for j, lo, hi in zip(QKV_TILES, project(2 * D, HD, ops), v_hi)}
        vs, after = {}, ks[7]
        for j in range(1, 8):
            t = jnp.where(lane_is(127, after), FILL[...].reshape(D // 8, 8, 128), vt[j].reshape(D // 8, 8, 128))
            vs[j] = after = pltpu.roll(t.reshape(D, 128), 1, 1)
        t = jnp.where(lane_is(-p, after), vt[0].reshape(D // 8, 8, 128), 0.0)
        FILL[...] = pltpu.roll(t.reshape(D, 128), 127, 1)
        outs = []
        for j in range(8):
            rows = []
            for hg in range(4):
                o = None
                for jj in QKV_TILES:
                    v = (vt if jj <= j else vs)[jj][hg * G:(hg + 1) * G]
                    t = v.reshape(DH, 8, 128) * probs[j, hg][(j - jj) % 8]
                    o = t if o is None else o + t
                rows.append(o.reshape(G, 128))
            outs.append(_cat(rows, 0))
        for j, r in zip(OUT_TILES, project(3 * D, D, pair_tiles([outs[j] for j in OUT_TILES]))):
            r = (r.reshape(D // 8, 8, 128) * peak[j]).reshape(D, 128)
            XP[p, j, xrows(0, D), :] = x = XP[p, j, xrows(0, D), :] + r
            put_stats(8 * p + j, 3, 0.5 * RHO if j % 2 else 0.5, x[0:1], *_moments(x, x[0:1]))

    def right_operands(p, t, r0):
        fs = [_forms(*(normed(p, 2 * t + hc, k * KB + r0, 16) for hc in range(2))) for k in range(3)]
        return [_combine(SCHEME[n][1], lambda f, k: fs[k][f]) for n in PRODUCTS]

    def prepare_ffn_input(i):
        r = pl.multiple_of(i * 16, 16)
        for t in range(4):
            for p in range(2):
                for q, v in enumerate(right_operands(p, t, r)):
                    RM[q, p, t, pl.ds(r, 16), :] = v.astype(bf16)
                src = r + 64 * (2 - p)
                for q, (own, v) in enumerate(zip(right_operands(p, t, src), right_operands(1 - p, t, src))):
                    RM[q, 2, t, pl.ds(r + 64 * p, 16), :] = own.astype(bf16)
                    RM[q, 1 - p, t, pl.ds(r + 64, 16), :] = (
                        v - RM[q, 2, t, pl.ds(r + 64 * p, 16), :].astype(f32)).astype(bf16)

    def gate_up_left(c, n):
        out = []
        for ref in (wg_raw, wu_raw):
            w = _combine(SCHEME[n][0], lambda i, k: ref[c, pl.ds(k * KB, KB), pl.ds(i * FT, FT)]).astype(bf16)
            out.append(_cat([w, w[128:KB]], 0).T)
        return _cat([w[r:r + 16] for r in range(0, FT, 16) for w in out], 0)

    def stage_left(c):
        for q in range(STAGED):
            A0[q] = pltpu.bitcast(gate_up_left(c, PRODUCTS[q]), i32)

    def gate_up(c):
        def glu(gu, scale):
            gu = gu.reshape(FT // 16, 2, 16, 128)
            return ((0.25 * jnp.tanh(_cat([scale, scale], 0) * gu[:, 0]) + 0.25) * gu[:, 1]).reshape(FT, 128)

        left = {}
        for q, n in enumerate(PRODUCTS):
            w = pltpu.bitcast(A0[q], bf16) if q < STAGED else gate_up_left(c + (c >> (5 + q)), n)
            both, second = _share_lhs(w[:, 0:128], w[:, 128:256], 2)
            left[n] = (w[:, 0:128], second, both)
        shared, products = {}, {}
        for t, g, n in _passes():
            m = _dot(left[n][g], RM[PRODUCTS.index(n), g, t])
            if g == 2:
                shared[t, n] = m
            else:
                products.setdefault((t, g), []).append((n, m + shared[t, n]))
        for (t, g), ms in products.items():
            sx, sy = ST[8 * g + 2 * t, 3] * 0.5, ST[8 * g + 2 * t + 1, 3] * (0.5 / RHO)
            fs = [_forms(glu(x, sx), glu(y, sy)) for x, y in _results(ms)]
            for q, n in enumerate(PRODUCTS):
                HS[q, 4 * g + t, pl.ds(pl.multiple_of(c * FT, FT), FT), :] = _combine(
                    SCHEME[n][1], lambda f, k: fs[k][f]).astype(bf16)
        stage_left(jnp.where(c == NCH - 1, 0, c + 1))

    def down(b):
        n = XB // 3
        r0 = pl.multiple_of(b * XB, XB)
        left = []
        for q, name in enumerate(PRODUCTS):
            z = b >> (5 + q)
            left.append(_combine(SCHEME[name][0], lambda i, k: _cat(
                [wd_raw[c + z, pl.ds(r0 + i * n, n), pl.ds(k * FT, FT)] for c in range(NCH)], 1)).astype(bf16))
        win = XP.at[:, :, pl.ds(r0, 2 * XB), :]
        finished = [win[t // 8, t % 8, 0:XB, :] for t in range(16)]
        cuts = (0, 4, 5, 6, 7, 8)
        for u0, u1 in zip(cuts[:-1], cuts[1:]):
            res = _results([(name, _dot(left[q], _cat([HS[q, u] for u in range(u0, u1)], 1)))
                            for q, name in enumerate(PRODUCTS)])
            for hc in range(2):
                y = _cat([ys[hc] for ys in res], 0)
                for u, dx in zip(range(u0, u1), _tiles([y])):
                    p, j = u // 4, 2 * (u % 4) + hc
                    t = 8 * p + j
                    dx = (dx.reshape(XB // 8, 8, 128) * (ST[t, 3] * (1 / RHO if hc else 1.0))).reshape(XB, 128)
                    win[p, j, XB:2 * XB, :] = x = win[p, j, XB:2 * XB, :] + dx
                    MOM[t, 0] = c = jnp.where(b == 0, jnp.broadcast_to(x[0:1], (16, 128)), MOM[t, 0])
                    for k, part in enumerate(_moments(x, c)):
                        MOM[t, 1 + k] = jnp.where(b == 0, 0.0, MOM[t, 1 + k]) + part
        return finished

    @pl.loop(0, 2)
    def _(layer):
        for t in range(16):
            put_stats(t, 2, 1.0, MOM[t, 0, 0:1, :], MOM[t, 1], MOM[t, 2])
        pl.loop(0, 2)(attention)

        @pl.when(layer == 0)
        def _():
            for cp in ffn_copies():
                cp.wait()
            stage_left(0)

        pl.loop(0, 4)(prepare_ffn_input)
        pl.loop(0, NCH)(gate_up)

        @pl.loop(0, NXB)
        def _(b):
            prev = jnp.maximum(b - 1, 0)
            finished = down(b)
            for part in range(2):
                store_rows(prev, part, [x[part * XB // 2:(part + 1) * XB // 2] for x in finished])

            @pl.when(jnp.logical_and(layer == 1, b > 0))
            def _():
                for part in range(2):
                    o_copy(prev, part).start()

    @pl.loop(0, 2)
    def _(part):
        rows = xrows(pl.multiple_of(D - XB + part * (XB // 2), XB // 2), XB // 2)
        store_rows(NXB - 1, part, [XP[t // 8, t % 8, rows, :] for t in range(16)])
        o_copy(NXB - 1, part).start()

    for b in range(NXB):
        for part in range(2):
            o_copy(b, part).wait()


@jax.jit
def pallas_interleave_layers__sliding_local_dilated__glu_gated_glu__prompt_kernel(
    A_x: jax.Array,
    A_wqkv: jax.Array,
    A_wo: jax.Array,
    B_x: jax.Array,
    B_w_gate: jax.Array,
    B_w_up: jax.Array,
    B_w_down: jax.Array,
):
    del B_x
    out = pl.pallas_call(
        _kernel,
        out_shape=jax.ShapeDtypeStruct((D, S), bf16),
        in_specs=[pl.BlockSpec(memory_space=pl.ANY)] * 6,
        out_specs=pl.BlockSpec(memory_space=pl.ANY),
        scratch_shapes=[
            pltpu.VMEM((6, 128, S), bf16),
            pltpu.VMEM((D, 3 * D), bf16),
            pltpu.VMEM((D, D), bf16),
            pltpu.VMEM((NCH, D, FC), bf16),
            pltpu.VMEM((NCH, D, FC), bf16),
            pltpu.VMEM((NCH, D, FC), bf16),
            pltpu.VMEM((2, S // 2 + 32, 128), i32),
            pltpu.VMEM((5, 3 * D + 32, 128), f32),
            pltpu.VMEM((6, 4 * HD, 128), i32),
            pltpu.VMEM((STAGED, FT, 256), i32),
            pltpu.VMEM((2, 8, XB + D, 128), f32),
            pltpu.VMEM((D, 128), f32),
            pltpu.VMEM((16, 3, 16, 128), f32),
            pltpu.VMEM((16, 4, 8, 128), f32),
            pltpu.VMEM((15, 3, 4, 128, 128), bf16),
            pltpu.VMEM((15, 8, F // 3, 128), bf16),
            pltpu.SemaphoreType.DMA((12,)),
        ],
        compiler_params=pltpu.CompilerParams(vmem_limit_bytes=120 * 2**20),
        name="interleave",
    )(A_x.reshape(S, D).T, A_wqkv, A_wo, B_w_gate, B_w_up, B_w_down.T)
    return out.T.reshape(1, S, D)
```

```python
import jax
import jax.numpy as jnp
import jax.experimental.pallas as pl
import jax.experimental.pallas.tpu as pltpu

S, D, F = 2048, 576, 4608
DH, WIN = 18, 8
G = 8 * DH
HD = D // 2
KB = D // 3
FT = 128
FC = 3 * FT
NCH = F // FC
XB = 192
NXB = D // XB
EPS = 1e-5
TINY = 1e-30
QKV_TILES = (1, 2, 3, 4, 5, 6, 7, 0)
OUT_TILES = (0, 7, 6, 1, 5, 2, 4, 3)
f32, bf16, i32 = jnp.float32, jnp.bfloat16, jnp.int32

RHO = 3 ** 0.5


def _scheme():
    out = {}
    for i in range(3):
        j, k = (i + 1) % 3, (i + 2) % 3
        for name, left, right, res in (
                ("a", [(1, i, j)], [(1, j, j), (-1, j, i)], [(1, i, i), (1, j, i)]),
                ("b", [(1, j, i)], [(1, i, i), (-1, i, j)], [(-1, j, j), (-1, i, j)]),
                ("c", [(1, i, j), (1, j, i)], [(1, i, j), (1, j, i)], [(-1, i, j), (1, j, i)]),
                ("d", [(1, i, i), (1, i, j), (-1, k, i)], [(1, j, i)], [(-1, i, k)]),
                ("e", [(1, i, i), (-1, j, i), (1, i, k)], [(1, k, i)], [(1, i, j)])):
            right = sorted(((-s if f == 2 else s, f, n) for s, f, n in right), key=lambda t: -t[0])
            if right[0][0] < 0:
                right, res = ([(-s, u, v) for s, u, v in ts] for ts in (right, res))
            out[name + str(i)] = (left, right, res)
    return out


SCHEME = _scheme()
STAGES = (("a0", "b0", "d0", "c0", "a2", "b2", "c2", "e0"), ("d1", "a1", "b1", "c1", "e1"), ("d2", "e2"))
PRODUCTS = [n for st in STAGES for n in st]
STAGED = 2


def _passes():
    order = []

    def run(t, g, stage):
        for n in STAGES[stage]:
            if (t, 2, n) not in order:
                order.append((t, 2, n))
            order.append((t, g, n))

    def shared(t, count):
        todo = [(t, 2, n) for n in PRODUCTS if t < 4 and (t, 2, n) not in order]
        order.extend(todo[:count])

    for t in range(4):
        run(t, 0, 0), run(t, 0, 1), shared(t + 1, 2), run(t, 0, 2)
        run(t, 1, 0), shared(t + 1, 1), run(t, 1, 1), shared(t + 1, 4), run(t, 1, 2)
    return order


def _dot(a, b):
    return jnp.dot(a, b, preferred_element_type=f32)


def _cat(xs, axis):
    return jnp.concatenate(xs, axis=axis)


def _tree(f, xs):
    while len(xs) > 1:
        xs = [f(xs[i], xs[i + 1]) for i in range(0, len(xs), 2)]
    return xs[0]


def _tiles(xs):
    return [x[:, i * 128:(i + 1) * 128] for x in xs for i in range(x.shape[1] // 128)]


def _combine(terms, block):
    v = block(*terms[0][1:])
    for s, *at in terms[1:]:
        v, w = v.astype(f32), block(*at).astype(f32)
        v = v + w if s > 0 else v - w
    return v


def _forms(x, y):
    return [x + y, x - y, x + x]


def _signed_sum(terms):
    s, v = terms[-1]
    for t, m in terms[-2::-1]:
        s, v = (s, v + m) if t == s else (1, v - m if s > 0 else m - v)
    return s, v


def _results(products):
    acc = {}
    for n, m in products:
        for s, i, d in SCHEME[n][2]:
            acc.setdefault((i, d), []).append((s, m))
    out = []
    for i in range(3):
        a = [_signed_sum(acc[i, d]) for d in range(3)]
        neg = [(-s, v) for s, v in a]
        x = _signed_sum([a[0], neg[1]])
        y = _signed_sum([_signed_sum([a[2], neg[1]]), _signed_sum([neg[0], a[2]])])
        assert x[0] == 1 and y[0] == 1
        out.append((x[1], y[1]))
    return out


def _share_lhs(last, tails, n):
    slot = jax.lax.broadcasted_iota(i32, (last.shape[0] // 2, 128), 1) // (128 // n)
    a, b = pltpu.bitcast(last, i32), pltpu.bitcast(tails, i32)
    return [pltpu.bitcast(jnp.where(slot == k, b, a), bf16) for k in range(n)]


def _share_mm(common, last, variants, rhs, shared):
    r = _dot(variants[0], shared)
    return [_dot(_cat([*common, w], 1), x) + r for w, x in zip([last, *variants[1:]], rhs)]


def _pow2(x):
    bits = pltpu.bitcast(jnp.clip(x, 2.0 ** -30, 2.0 ** 30), i32) & 0x7F800000
    return pltpu.bitcast(bits, f32), pltpu.bitcast(0x7F000000 - bits, f32)


def _moments(x, c):
    xc = x.reshape(x.shape[0] // 16, 16, 128) - c
    return jnp.sum(xc, axis=0), jnp.sum(xc * xc, axis=0)


def _kernel(x_hbm, wqkv_hbm, wo_hbm, wg_hbm, wu_hbm, wd_hbm, o_hbm,
            xio, wqkv_raw, wo_raw, wg_raw, wu_raw, wd_raw, words, tmp,
            WT, A0, XP, FILL, MOM, ST, SC, RM, HS, balanced, sems):
    def xrows(r0, n):
        return pl.ds(XB + r0, n)

    def ffn_copies():
        return [pltpu.make_async_copy(src.at[:, pl.ds(c * FC, FC)], dst.at[c], sems.at[11])
                for c in range(NCH)
                for src, dst in ((wg_hbm, wg_raw), (wu_hbm, wu_raw), (wd_hbm, wd_raw))]

    def x_copy(b, n):
        return pltpu.make_async_copy(x_hbm.at[pl.ds(b * 128, n), :], xio.at[b, pl.ds(0, n), :], sems.at[b])

    def w_copy(kt, n):
        rows = pl.ds(pl.multiple_of(kt * 128, 128), n)
        return pltpu.make_async_copy(wqkv_hbm.at[rows, :], wqkv_raw.at[rows, :], sems.at[5 + kt])

    def o_copy(b, part):
        k, n = 2 * b + part, XB // 2
        return pltpu.make_async_copy(xio.at[k, pl.ds(0, n), :], o_hbm.at[pl.ds(k * n, n), :], sems.at[k])

    wo_copy = pltpu.make_async_copy(wo_hbm, wo_raw, sems.at[10])
    x_copy(4, 64).start()
    for b in range(4):
        x_copy(b, 128).start()
    w_copy(4, 64).start()
    wo_copy.start()
    for kt in (3, 0, 1, 2):
        w_copy(kt, 128).start()

    FILL[...] = jnp.zeros(FILL.shape, f32)
    SC[...] = jnp.ones(SC.shape, f32)

    @pl.loop(0, 8)
    def _(j):
        XP[:, j, 0:XB, :] = jnp.zeros((2, XB, 128), f32)

    def load_rows(b, n, first):
        x_copy(b, n).wait()
        words[0, 0:S // 2, 0:n] = pltpu.bitcast(xio[b, pl.ds(0, n), :].T, i32)
        for j in range(8):
            pair = words[0, pl.ds(j, 128, stride=8), pl.ds(0, n)].T
            for p, bits in enumerate((pair << 16, pair & -65536)):
                x = pltpu.bitcast(bits, f32)
                XP[p, j, xrows(pl.multiple_of(b * 128, 128), n), :] = x
                t = 8 * p + j
                if first:
                    MOM[t, 0] = c = jnp.broadcast_to(x[0:1], (16, 128))
                    MOM[t, 1], MOM[t, 2] = _moments(x, c)
                else:
                    s1, s2 = _moments(x, MOM[t, 0])
                    MOM[t, 1] += s1
                    MOM[t, 2] += s2

    def store_rows(b, part, xs):
        n = XB // 2
        for j in range(8):
            lo, hi = (pltpu.bitcast(xs[8 * p + j].astype(bf16).astype(f32), i32) for p in range(2))
            words[part, pl.ds(j, 128, stride=8), pl.ds(0, n)] = (jax.lax.shift_right_logical(lo, 16) | hi).T
        xio[2 * b + part, pl.ds(0, n), :] = pltpu.bitcast(words[part, 0:S // 2, 0:n], bf16).T

    def regroup(t, groups, n):
        return _cat([tmp[t, pl.ds(g * G + d, 8, stride=DH), pl.ds(0, n)]
                     for g in range(groups) for d in range(DH)], 0)

    def prepare_wqkv(kt, n=128, last=False):
        w_copy(kt, n).wait()
        w = wqkv_raw[pl.ds(pl.multiple_of(kt * 128, 128), n), :]
        tmp[0, 0:3 * D, :] = _cat([w] * (128 // n), 0).astype(f32).T
        wt = regroup(0, 12, 128).astype(bf16)
        WT[kt, pl.ds(0, 3 * HD), :] = pltpu.bitcast(wt, i32)
        if last:
            for k, v in enumerate(_share_lhs(wt, pltpu.bitcast(WT[4, pl.ds(0, 3 * HD), :], bf16), 2)):
                WT[4 + k, pl.ds(0, 3 * HD), :] = pltpu.bitcast(v, i32)

    def prepare_wo():
        wo_copy.wait()
        cols = [(ct, min(128, D - ct * 128)) for ct in range(5)]
        for ct, n in cols:
            tmp[ct, 0:D, 0:n] = wo_raw[:, pl.ds(ct * 128, n)].astype(f32)
        for ct, n in cols:
            rows = regroup(ct, 4, n)
            rows = _cat([rows, rows[448:512], rows[384:448], rows[512:576]], 0)
            for kt in range(6):
                WT[kt, pl.ds(3 * HD + ct * 64, n // 2), :] = pltpu.bitcast(
                    rows[kt * 128:(kt + 1) * 128].T.astype(bf16), i32)

    load_rows(4, 64, True)
    pl.loop(0, 4)(lambda b: load_rows(b, 128, False))
    prepare_wqkv(4, 64)
    prepare_wo()
    prepare_wqkv(3, last=True)
    pl.loop(0, 3)(prepare_wqkv)
    for cp in ffn_copies():
        cp.start()

    def put_stats(t, slot, scale, c, s1, s2):
        m = jnp.sum(s1, axis=0, keepdims=True) * (1.0 / D)
        v = jnp.maximum(jnp.sum(s2, axis=0, keepdims=True) * (1.0 / D) - m * m, 0.0)
        unit = jax.lax.rsqrt(v + TINY)
        ST[t, 0] = jnp.broadcast_to(c + m, (8, 128))
        ST[t, 1] = jnp.broadcast_to(unit * scale, (8, 128))
        ST[t, slot] = jnp.broadcast_to((v + TINY) * unit * jax.lax.rsqrt(v + EPS), (8, 128))

    def normed(p, j, r0, n):
        x = XP[p, j, xrows(r0, n), :].reshape(n // 8, 8, 128)
        return ((x - ST[8 * p + j, 0]) * ST[8 * p + j, 1]).reshape(n, 128)

    def pair_tiles(ts):
        xa, xb = _cat(ts[0:4], 1), _cat(ts[4:8], 1)
        ra, rb = xa[512:576].astype(bf16).astype(f32), xb[448:512].astype(bf16).astype(f32)
        pa = _cat([xa[0:448], xa[448:512] - rb], 0).astype(bf16)
        pb = _cat([xb[0:448], xb[512:576] - ra], 0).astype(bf16)
        return [pa, pb], _cat([xa[512:576], xb[448:512]], 0).astype(bf16)

    def project(r0, n, ops):
        w = [pltpu.bitcast(WT[kt, pl.ds(r0 // 2, n // 2), :], bf16) for kt in range(6)]
        return _tiles(_share_mm(w[0:3], w[3], w[4:6], *ops))

    def attention(p):
        lane = jax.lax.broadcasted_iota(i32, (8, 128), 1)

        def lane_is(at, after):
            return lane + (pltpu.bitcast(after[D - 8:D], i32) & (p >> 4)) == at

        ops = pair_tiles([normed(p, j, 0, D) for j in QKV_TILES])
        kt = dict(zip(QKV_TILES, project(D, D, ops)))
        ks = {j: pltpu.roll(kt[j], 1, 1) for j in range(1, 8)}
        v_hi = project(2 * D + HD, HD, ops)
        gt = [ST[8 * p + j, 2] for j in range(8)]
        gz = {j: jnp.where(lane == 0, 0.0, pltpu.roll(gt[j], 1, 1)) for j in range(1, 8)}
        gs = {j: jnp.where(lane == 0, ST[0, 2], g) for j, g in gz.items()}
        probs, peak = {}, {}
        for j, q in zip(QKV_TILES, project(0, D, ops)):
            gains = [(gt if j >= w else gs)[(j - w) % 8] for w in range(WIN)]
            scales = [g * (gt[j] * DH ** -0.5) for g in gains]
            peak[j] = _tree(jnp.maximum, [(gt if j >= w else gz)[(j - w) % 8] for w in range(WIN)])
            gains = [g * (1.0 / peak[j]) for g in gains]
            for hg in range(4):
                logits = []
                for w in range(WIN):
                    t = q[hg * G:(hg + 1) * G] * (kt if j >= w else ks)[(j - w) % 8][hg * G:(hg + 1) * G]
                    lg = jnp.sum(t.reshape(DH, 8, 128), axis=0) * scales[w]
                    logits.append(lg if j >= w else jnp.where(lane == 0, -1e9, lg))
                m = _tree(jnp.maximum, logits)
                es = [jnp.exp(lg - m) for lg in logits]
                inv = 1.0 / _tree(jnp.add, es)
                if j < 7:
                    es[j] = es[j] + jnp.where(lane + p == 0, (7 - j) * es[7], 0.0)
                probs[j, hg] = [e * inv * g for e, g in zip(es, gains)]
        vt = {j: _cat([lo, hi], 0) for j, lo, hi in zip(QKV_TILES, project(2 * D, HD, ops), v_hi)}
        vs, after = {}, ks[7]
        for j in range(1, 8):
            t = jnp.where(lane_is(127, after), FILL[...].reshape(D // 8, 8, 128), vt[j].reshape(D // 8, 8, 128))
            vs[j] = after = pltpu.roll(t.reshape(D, 128), 1, 1)
        t = jnp.where(lane_is(-p, after), vt[0].reshape(D // 8, 8, 128), 0.0)
        FILL[...] = pltpu.roll(t.reshape(D, 128), 127, 1)
        outs = []
        for j in range(8):
            rows = []
            for hg in range(4):
                o = None
                for jj in QKV_TILES:
                    v = (vt if jj <= j else vs)[jj][hg * G:(hg + 1) * G]
                    t = v.reshape(DH, 8, 128) * probs[j, hg][(j - jj) % 8]
                    o = t if o is None else o + t
                rows.append(o.reshape(G, 128))
            outs.append(_cat(rows, 0))
        for j, r in zip(OUT_TILES, project(3 * D, D, pair_tiles([outs[j] for j in OUT_TILES]))):
            r = (r.reshape(D // 8, 8, 128) * peak[j]).reshape(D, 128)
            XP[p, j, xrows(0, D), :] = x = XP[p, j, xrows(0, D), :] + r
            put_stats(8 * p + j, 3, 0.5 * RHO if j % 2 else 0.5, x[0:1], *_moments(x, x[0:1]))

    def balance_weights():
        def size(x):
            return jnp.abs(x.astype(f32))

        def rows(i):
            return pl.ds(pl.multiple_of(i * 32, 32), 32)

        def unit_sizes(c):
            return jnp.sum(size(wu_raw[c]), axis=0, keepdims=True)

        ones = jnp.ones((128, 128), bf16)
        samples = [_dot(size(ref[0, :, 0:128]).astype(bf16), ones) for ref in (wg_raw, wu_raw, wd_raw)]
        hi = [jnp.max(v, axis=0, keepdims=True) for v in samples]
        lo = [jnp.min(v, axis=0, keepdims=True) for v in samples]
        units = _tiles([jnp.sum(size(wu_raw[c, 0:64, :]), axis=0, keepdims=True) for c in range(NCH)])
        hi.append(jnp.max(_cat(units, 0), axis=0, keepdims=True))
        lo.append(jnp.min(_cat(units, 0), axis=0, keepdims=True))
        stage_left(0)
        uneven = jnp.max(_tree(jnp.maximum, [a - 4.0 * b for a, b in zip(hi, lo)])) > 0.0
        balanced[0] = uneven.astype(i32)

        @pl.when(uneven)
        def _():
            total = jax.lax.fori_loop(0, NCH, lambda c, t: t + unit_sizes(c), jnp.zeros((1, FC), f32))
            mean = jnp.maximum(jnp.sum(total, axis=1, keepdims=True) * (1.0 / F), TINY)

            @pl.loop(0, NCH)
            def _(c):
                up, inv = _pow2(unit_sizes(c) / mean)

                @pl.loop(0, D // 32)
                def _(i):
                    for ref, factor in ((wu_raw, inv), (wd_raw, up)):
                        ref[c, rows(i), :] = (ref[c, rows(i), :].astype(f32) * factor).astype(bf16)

            def row_sizes(i, totals):
                out = []
                for n, ref in enumerate((wg_raw, wu_raw, wd_raw)):
                    v = jax.lax.fori_loop(0, NCH, lambda c, t: t + size(ref[c, rows(i), :]), jnp.zeros((32, FC), f32))
                    tmp[n, rows(i), :] = v = jnp.broadcast_to(jnp.sum(v, axis=1, keepdims=True), (32, 128))
                    out.append(totals[n] + jnp.sum(v, axis=0, keepdims=True) * (1.0 / D))
                return out

            means = jax.lax.fori_loop(0, D // 32, row_sizes, [jnp.zeros((1, 128), f32)] * 3)

            @pl.loop(0, D // 32)
            def _(i):
                g, u, d = (tmp[n, rows(i), :] / jnp.maximum(means[n], TINY) for n in range(3))
                (SC[0, rows(i), :], inv_in), (SC[1, rows(i), :], inv_out) = _pow2(g + u), _pow2(d)

                @pl.loop(0, NCH)
                def _(c):
                    for ref, factor in ((wg_raw, inv_in), (wu_raw, inv_in), (wd_raw, inv_out)):
                        ref[c, rows(i), :] = (ref[c, rows(i), :].astype(f32) * _cat([factor] * 3, 1)).astype(bf16)

            stage_left(0)

    def prepare_ffn_input(i, scaled):
        def block(p, j, r0):
            x = normed(p, j, r0, 16)
            return x * SC[0, pl.ds(r0, 16), :] if scaled else x

        def right_operands(p, t, r0):
            fs = [_forms(*(block(p, 2 * t + hc, k * KB + r0) for hc in range(2))) for k in range(3)]
            return [_combine(SCHEME[n][1], lambda f, k: fs[k][f]) for n in PRODUCTS]

        r = pl.multiple_of(i * 16, 16)
        for t in range(4):
            for p in range(2):
                for q, v in enumerate(right_operands(p, t, r)):
                    RM[q, p, t, pl.ds(r, 16), :] = v.astype(bf16)
                src = r + 64 * (2 - p)
                for q, (own, v) in enumerate(zip(right_operands(p, t, src), right_operands(1 - p, t, src))):
                    RM[q, 2, t, pl.ds(r + 64 * p, 16), :] = own.astype(bf16)
                    RM[q, 1 - p, t, pl.ds(r + 64, 16), :] = (
                        v - RM[q, 2, t, pl.ds(r + 64 * p, 16), :].astype(f32)).astype(bf16)

    def gate_up_left(c, n):
        out = []
        for ref in (wg_raw, wu_raw):
            w = _combine(SCHEME[n][0], lambda i, k: ref[c, pl.ds(k * KB, KB), pl.ds(i * FT, FT)]).astype(bf16)
            out.append(_cat([w, w[128:KB]], 0).T)
        return _cat([w[r:r + 16] for r in range(0, FT, 16) for w in out], 0)

    def stage_left(c):
        for q in range(STAGED):
            A0[q] = pltpu.bitcast(gate_up_left(c, PRODUCTS[q]), i32)

    def gate_up(c):
        def glu(gu, scale):
            gu = gu.reshape(FT // 16, 2, 16, 128)
            return ((0.25 * jnp.tanh(_cat([scale, scale], 0) * gu[:, 0]) + 0.25) * gu[:, 1]).reshape(FT, 128)

        left = {}
        for q, n in enumerate(PRODUCTS):
            w = pltpu.bitcast(A0[q], bf16) if q < STAGED else gate_up_left(c + (c >> (5 + q)), n)
            both, second = _share_lhs(w[:, 0:128], w[:, 128:256], 2)
            left[n] = (w[:, 0:128], second, both)
        shared, products = {}, {}
        for t, g, n in _passes():
            m = _dot(left[n][g], RM[PRODUCTS.index(n), g, t])
            if g == 2:
                shared[t, n] = m
            else:
                products.setdefault((t, g), []).append((n, m + shared[t, n]))
        for (t, g), ms in products.items():
            sx, sy = ST[8 * g + 2 * t, 3] * 0.5, ST[8 * g + 2 * t + 1, 3] * (0.5 / RHO)
            fs = [_forms(glu(x, sx), glu(y, sy)) for x, y in _results(ms)]
            for q, n in enumerate(PRODUCTS):
                HS[q, 4 * g + t, pl.ds(pl.multiple_of(c * FT, FT), FT), :] = _combine(
                    SCHEME[n][1], lambda f, k: fs[k][f]).astype(bf16)
        stage_left(jnp.where(c == NCH - 1, 0, c + 1))

    def down(b):
        n = XB // 3
        r0 = pl.multiple_of(b * XB, XB)
        left = []
        for q, name in enumerate(PRODUCTS):
            z = b >> (5 + q)
            left.append(_combine(SCHEME[name][0], lambda i, k: _cat(
                [wd_raw[c + z, pl.ds(r0 + i * n, n), pl.ds(k * FT, FT)] for c in range(NCH)], 1)).astype(bf16))
        win = XP.at[:, :, pl.ds(r0, 2 * XB), :]
        finished = [win[t // 8, t % 8, 0:XB, :] for t in range(16)]
        cuts = (0, 4, 5, 6, 7, 8)
        for u0, u1 in zip(cuts[:-1], cuts[1:]):
            res = _results([(name, _dot(left[q], _cat([HS[q, u] for u in range(u0, u1)], 1)))
                            for q, name in enumerate(PRODUCTS)])
            for hc in range(2):
                y = _cat([ys[hc] for ys in res], 0)
                for u, dx in zip(range(u0, u1), _tiles([y])):
                    p, j = u // 4, 2 * (u % 4) + hc
                    t = 8 * p + j
                    dx = dx * SC[1, pl.ds(r0, XB), :]
                    dx = (dx.reshape(XB // 8, 8, 128) * (ST[t, 3] * (1 / RHO if hc else 1.0))).reshape(XB, 128)
                    win[p, j, XB:2 * XB, :] = x = win[p, j, XB:2 * XB, :] + dx
                    MOM[t, 0] = c = jnp.where(b == 0, jnp.broadcast_to(x[0:1], (16, 128)), MOM[t, 0])
                    for k, part in enumerate(_moments(x, c)):
                        MOM[t, 1 + k] = jnp.where(b == 0, 0.0, MOM[t, 1 + k]) + part
        return finished

    @pl.loop(0, 2)
    def _(layer):
        for t in range(16):
            put_stats(t, 2, 1.0, MOM[t, 0, 0:1, :], MOM[t, 1], MOM[t, 2])
        pl.loop(0, 2)(attention)

        @pl.when(layer == 0)
        def _():
            for cp in ffn_copies():
                cp.wait()
            balance_weights()

        for scaled in range(2):
            @pl.when(balanced[0] == scaled)
            def _():
                pl.loop(0, 4)(lambda i: prepare_ffn_input(i, scaled))

        pl.loop(0, NCH)(gate_up)

        @pl.loop(0, NXB)
        def _(b):
            prev = jnp.maximum(b - 1, 0)
            finished = down(b)
            for part in range(2):
                store_rows(prev, part, [x[part * XB // 2:(part + 1) * XB // 2] for x in finished])

            @pl.when(jnp.logical_and(layer == 1, b > 0))
            def _():
                for part in range(2):
                    o_copy(prev, part).start()

    @pl.loop(0, 2)
    def _(part):
        rows = xrows(pl.multiple_of(D - XB + part * (XB // 2), XB // 2), XB // 2)
        store_rows(NXB - 1, part, [XP[t // 8, t % 8, rows, :] for t in range(16)])
        o_copy(NXB - 1, part).start()

    for b in range(NXB):
        for part in range(2):
            o_copy(b, part).wait()


@jax.jit
def pallas_interleave_layers__sliding_local_dilated__glu_gated_glu__prompt_kernel(
    A_x: jax.Array,
    A_wqkv: jax.Array,
    A_wo: jax.Array,
    B_x: jax.Array,
    B_w_gate: jax.Array,
    B_w_up: jax.Array,
    B_w_down: jax.Array,
):
    del B_x
    out = pl.pallas_call(
        _kernel,
        out_shape=jax.ShapeDtypeStruct((D, S), bf16),
        in_specs=[pl.BlockSpec(memory_space=pl.ANY)] * 6,
        out_specs=pl.BlockSpec(memory_space=pl.ANY),
        scratch_shapes=[
            pltpu.VMEM((6, 128, S), bf16),
            pltpu.VMEM((D, 3 * D), bf16),
            pltpu.VMEM((D, D), bf16),
            pltpu.VMEM((NCH, D, FC), bf16),
            pltpu.VMEM((NCH, D, FC), bf16),
            pltpu.VMEM((NCH, D, FC), bf16),
            pltpu.VMEM((2, S // 2 + 32, 128), i32),
            pltpu.VMEM((5, 3 * D + 32, 128), f32),
            pltpu.VMEM((6, 4 * HD, 128), i32),
            pltpu.VMEM((STAGED, FT, 256), i32),
            pltpu.VMEM((2, 8, XB + D, 128), f32),
            pltpu.VMEM((D, 128), f32),
            pltpu.VMEM((16, 3, 16, 128), f32),
            pltpu.VMEM((16, 4, 8, 128), f32),
            pltpu.VMEM((2, D, 128), f32),
            pltpu.VMEM((15, 3, 4, 128, 128), bf16),
            pltpu.VMEM((15, 8, F // 3, 128), bf16),
            pltpu.SMEM((1,), i32),
            pltpu.SemaphoreType.DMA((12,)),
        ],
        compiler_params=pltpu.CompilerParams(vmem_limit_bytes=120 * 2**20),
        name="interleave",
    )(A_x.reshape(S, D).T, A_wqkv, A_wo, B_w_gate, B_w_up, B_w_down.T)
    return out.T.reshape(1, S, D)
```
